```python
import os as _os
_os.environ.setdefault("JAX_PLATFORMS", "cpu")
import jax
import jax.numpy as jnp

def _softmax(x, axis=-1):
    return jax.nn.softmax(x, axis=axis)
def _gelu(x):
    return jax.nn.gelu(x, approximate=True)
def _silu(x):
    return jax.nn.silu(x)
def _sigmoid(x):
    return jax.nn.sigmoid(x)
def _layernorm(x, axis=-1, eps=1e-5):
    m = jnp.mean(x, axis=axis, keepdims=True)
    v = jnp.var(x, axis=axis, keepdims=True)
    return (x - m) / jnp.sqrt(v + eps)
def _scatter_add(tgt, idx, src, axis=0):
    return tgt.at[idx].add(src)
def _segment_sum(src, seg, n):
    return jax.ops.segment_sum(src, seg, n)
class _Rng:
    def __init__(self, key):
        self._k = key
    def _next(self):
        self._k, sub = jax.random.split(self._k)
        return sub
    def normal(self, shape):
        return jax.random.normal(self._next(), shape, dtype=jnp.bfloat16)
    def randint(self, lo, hi, shape):
        return jax.random.randint(self._next(), shape, lo, hi, dtype=jnp.int32)
    def uniform(self, shape, lo=0.0, hi=1.0):
        return jax.random.uniform(self._next(), shape, jnp.bfloat16, lo, hi)
    def permutation(self, n):
        return jax.random.permutation(self._next(), n)


kernel_name = 'concat_heads__gqa_block_cached__gqa_block_cached__near_ridge'

def setup_inputs():
    _rng = _Rng(jax.random.key(int.from_bytes(__import__("os").urandom(4), "little")))
    _w = (lambda a: (lambda t: t.astype(jnp.bfloat16) if jnp.issubdtype(t.dtype, jnp.floating) else t)(jnp.asarray(a)))
    def _A_setup():
        B, Sq, D = 32, 48, 512
        Hq, Hkv, Sk, Dh = 32, 32, 48, 128
        assert Hq % Hkv == 0, (Hq, Hkv)
        return {
            "x": _w((lambda *s: _rng.normal(s) * 0.8)(B, Sq, D)),
            "k_cache": _w((lambda *s: _rng.normal(s) * 0.8)(B, Hkv, Sk, Dh)),
            "v_cache": _w((lambda *s: _rng.normal(s) * 0.05)(B, Hkv, Sk, Dh)),
            "wq": _w((lambda *s: _rng.normal(s) * 0.8)(D, Hq * Dh) * (D ** -0.5)),
            "wo": _w((lambda *s: _rng.normal(s) * 0.05)(Hq * Dh, D) * ((Hq * Dh) ** -0.5)),
        }
    _A_in = _A_setup()

    def _B_setup():
        B, Sq, D = 32, 48, 512
        Hq, Hkv, Sk, Dh = 32, 32, 48, 128
        assert Hq % Hkv == 0, (Hq, Hkv)
        return {
            "x": _w((lambda *s: _rng.normal(s) * 0.8)(B, Sq, D)),
            "k_cache": _w((lambda *s: _rng.normal(s) * 0.8)(B, Hkv, Sk, Dh)),
            "v_cache": _w((lambda *s: _rng.normal(s) * 0.05)(B, Hkv, Sk, Dh)),
            "wq": _w((lambda *s: _rng.normal(s) * 0.8)(D, Hq * Dh) * (D ** -0.5)),
            "wo": _w((lambda *s: _rng.normal(s) * 0.05)(Hq * Dh, D) * ((Hq * Dh) ** -0.5)),
        }
    _B_in = _B_setup()

    return {
        "A_x": _A_in["x"],
        "A_k_cache": _A_in["k_cache"],
        "A_v_cache": _A_in["v_cache"],
        "A_wq": _A_in["wq"],
        "A_wo": _A_in["wo"],
        "B_x": _B_in["x"],
        "B_k_cache": _B_in["k_cache"],
        "B_v_cache": _B_in["v_cache"],
        "B_wq": _B_in["wq"],
        "B_wo": _B_in["wo"],
    }

def reference(A_x, A_k_cache, A_v_cache, A_wq, A_wo, B_x, B_k_cache, B_v_cache, B_wq, B_wo):
    def _A_ref(x, k_cache, v_cache, wq, wo):
        B, Sq, D = x.shape
        Hq, Dh = 32, 128
        Hkv = k_cache.shape[1]
        rep = Hq // Hkv
        q = (lambda x, *d: x.transpose(*d))((x @ wq).reshape(B, Sq, Hq, Dh), 0, 2, 1, 3)
        k = jnp.repeat(k_cache, rep, axis=1)
        v = jnp.repeat(v_cache, rep, axis=1)
        scores = jnp.einsum("bhqd,bhkd->bhqk", q, k) * (Dh ** -0.5)
        p = _softmax(scores, axis=-1)
        o = jnp.einsum("bhqk,bhkd->bhqd", p, v)
        return (lambda x, *d: x.transpose(*d))(o, 0, 2, 1, 3).reshape(B, Sq, Hq * Dh) @ wo

    def _B_ref(x, k_cache, v_cache, wq, wo):
        B, Sq, D = x.shape
        Hq, Dh = 32, 128
        Hkv = k_cache.shape[1]
        rep = Hq // Hkv
        q = (lambda x, *d: x.transpose(*d))((x @ wq).reshape(B, Sq, Hq, Dh), 0, 2, 1, 3)
        k = jnp.repeat(k_cache, rep, axis=1)
        v = jnp.repeat(v_cache, rep, axis=1)
        scores = jnp.einsum("bhqd,bhkd->bhqk", q, k) * (Dh ** -0.5)
        p = _softmax(scores, axis=-1)
        o = jnp.einsum("bhqk,bhkd->bhqd", p, v)
        return (lambda x, *d: x.transpose(*d))(o, 0, 2, 1, 3).reshape(B, Sq, Hq * Dh) @ wo

    a = _A_ref(A_x, A_k_cache, A_v_cache, A_wq, A_wo)
    b = _B_ref(B_x, B_k_cache, B_v_cache, B_wq, B_wo)
    return jnp.concatenate([a, b], axis=-1)
```

```python
import math

import jax
import jax.numpy as jnp
from jax import lax
import jax.experimental.pallas as pl
import jax.experimental.pallas.tpu as pltpu

_NT = (((1,), (1,)), ((), ()))


@jax.jit
def pallas_concat_heads__gqa_block_cached__gqa_block_cached__near_ridge_kernel(
    A_x: jax.Array,
    A_k_cache: jax.Array,
    A_v_cache: jax.Array,
    A_wq: jax.Array,
    A_wo: jax.Array,
    B_x: jax.Array,
    B_k_cache: jax.Array,
    B_v_cache: jax.Array,
    B_wq: jax.Array,
    B_wo: jax.Array,
):
    B, S, D = A_x.shape
    _, H, _, DH = A_k_cache.shape
    M = B * S
    G, PB = 1, 2
    NG = H // G
    R = PB * S
    NP = B // PB
    c = (DH ** -0.5) * math.log2(math.e)

    def qproj(x_ref, wq_ref):
        q = jnp.dot(x_ref[...], wq_ref[...], preferred_element_type=jnp.float32)
        return q.astype(jnp.bfloat16)

    def unit(qh, kk, vv, mask):
        s = lax.dot_general(qh, kk, _NT, preferred_element_type=jnp.float32)
        s = jnp.where(mask, s, -jnp.inf)
        m = jnp.max(s, axis=-1, keepdims=True)
        e = jnp.exp2((s - m) * c)
        l = jnp.sum(e, axis=-1, keepdims=True)
        o = jnp.dot(e.astype(jnp.bfloat16), vv, preferred_element_type=jnp.float32)
        return (o * pl.reciprocal(l, approx=True)).astype(jnp.bfloat16)

    def attn(q, k_ref, v_ref, mask):
        rows = []
        for p in range(NP):
            qh = q[p * R:(p + 1) * R, :]
            kk = k_ref[p * PB:(p + 1) * PB, 0].reshape(R, DH)
            vv = v_ref[p * PB:(p + 1) * PB, 0].reshape(R, DH)
            rows.append(unit(qh, kk, vv, mask))
        return jnp.concatenate(rows, axis=0)

    def oproj(o, wo_ref, acc_ref, col):
        acc_ref[:, col:col + D] += jnp.dot(o, wo_ref[...], preferred_element_type=jnp.float32)

    def kernel(ax, ak, av, awq, awo, bx, bk, bv, bwq, bwo, out_ref, acc_ref):
        g = pl.program_id(0)

        @pl.when(g == 0)
        def _():
            acc_ref[...] = jnp.zeros_like(acc_ref)

        ri = lax.broadcasted_iota(jnp.int32, (R, R), 0) // S
        ci = lax.broadcasted_iota(jnp.int32, (R, R), 1) // S
        mask = ri == ci
        qa = qproj(ax, awq)
        qb = qproj(bx, bwq)
        oa = attn(qa, ak, av, mask)
        ob = attn(qb, bk, bv, mask)
        oproj(oa, awo, acc_ref, 0)
        oproj(ob, bwo, acc_ref, D)

        @pl.when(g == NG - 1)
        def _():
            out_ref[...] = acc_ref[...].astype(out_ref.dtype)

    xs = pl.BlockSpec((M, D), lambda g: (0, 0))
    kvs = pl.BlockSpec((B, G, S, DH), lambda g: (0, g, 0, 0))
    wqs = pl.BlockSpec((D, G * DH), lambda g: (0, g))
    wos = pl.BlockSpec((G * DH, D), lambda g: (g, 0))
    out = pl.pallas_call(
        kernel,
        grid=(NG,),
        in_specs=[xs, kvs, kvs, wqs, wos] * 2,
        out_specs=pl.BlockSpec((M, 2 * D), lambda g: (0, 0)),
        out_shape=jax.ShapeDtypeStruct((M, 2 * D), A_x.dtype),
        scratch_shapes=[pltpu.VMEM((M, 2 * D), jnp.float32)],
        compiler_params=pltpu.CompilerParams(
            dimension_semantics=("arbitrary",),
            vmem_limit_bytes=64 * 1024 * 1024,
        ),
    )(A_x.reshape(M, D), A_k_cache, A_v_cache, A_wq, A_wo,
      B_x.reshape(M, D), B_k_cache, B_v_cache, B_wq, B_wo)
    return out.reshape(B, S, 2 * D)
```

```python
import math
import jax, jax.numpy as jnp
from jax import lax
import jax.experimental.pallas as pl
import jax.experimental.pallas.tpu as pltpu

B, S, D, H, DH = 32, 48, 512, 32, 128
M = B * S
NT_DIMS = (((1,), (1,)), ((), ()))
F32 = jnp.float32
BF = jnp.bfloat16

def build(G=4, CS=2, NC=4, PB=2, nobc=False, nosc=False, OSUB=1, QW=4):
    NG = H // G
    NT = 2 * NG
    c = (DH ** -0.5) * math.log2(math.e)
    R = PB * S
    RB = B // NC
    MC = RB * S
    NPC = RB // PB
    GW = G * DH
    NO = NC * OSUB
    MO = M // NO

    def kernel(ax, ak, av, awq, awo, bx, bk, bv, bwq, bwo, out_hbm,
               x_s, k_s, v_s, wq_s, wo_s, acc, out_s, sems):
        src = ((ax, ak, av, awq, awo), (bx, bk, bv, bwq, bwo))

        def x_dma(br, lo, n, sem):
            return pltpu.make_async_copy(src[br][0].at[pl.ds(lo, n)], x_s.at[br, pl.ds(lo, n)], sems.at[sem])
        def kv_dma(which, t, sem):
            br, g = divmod(t, NG) if isinstance(t, int) else (0, 0)
            return pltpu.make_async_copy(src[br][1 + which].at[:, pl.ds(g * G, G)], (k_s, v_s)[which].at[t], sems.at[sem])
        def wq_dma(t, sem, h0=0, nh=G):
            br, g = divmod(t, NG) if isinstance(t, int) else (0, 0)
            return pltpu.make_async_copy(src[br][3].at[:, pl.ds(g * GW + h0 * DH, nh * DH)], wq_s.at[t, :, pl.ds(h0 * DH, nh * DH)], sems.at[sem])
        def wo_dma(t, sem):
            br, g = divmod(t, NG) if isinstance(t, int) else (0, 0)
            return pltpu.make_async_copy(src[br][4].at[pl.ds(g * GW, GW), :], wo_s.at[t], sems.at[sem])
        def out_dma(br, oi):
            return pltpu.make_async_copy(out_s.at[br, pl.ds(oi * MO, MO)],
                                         out_hbm.at[pl.ds(oi * MO, MO), pl.ds(br * D, D)], sems.at[SEM_OUT + br])

        SEM_STEP0 = 0
        SEM_XB = NT
        SEM_OUT = NT + 1
        SEM_COLD = NT + 3
        pieces = []
        for t in range(CS):
            for h0 in range(0, G, QW):
                pieces.append((t, h0, QW))
        groups = []
        groups.append([('wq',) + pieces[0], ('x', 0)])
        groups.append([('x', 1), ('x', 2)])
        groups.append([('x', 3)] + ([('wq',) + pieces[1]] if len(pieces) > 1 else []))
        if len(pieces) > 2:
            groups.append([('wq',) + p for p in pieces[2:]])
        def mk(item, sem):
            if item[0] == 'wq': return wq_dma(item[1], sem, item[2], item[3])
            if item[0] == 'x': return x_dma(0, item[1] * MC, MC, sem)
        cold_dmas = [[mk(it, SEM_COLD + gi) for it in grp] for gi, grp in enumerate(groups)]
        def step_dmas(t, with_wq):
            l = []
            if with_wq: l.append(wq_dma(t, t))
            l += [kv_dma(0, t, t), kv_dma(1, t, t), wo_dma(t, t)]
            return l
        for grp in cold_dmas:
            for d in grp: d.start()
        for t in range(NT):
            if t == NG:
                x_dma(1, 0, M, SEM_XB).start(priority=1)
            for d in step_dmas(t, t >= CS): d.start(priority=1)

        ri = lax.broadcasted_iota(jnp.int32, (R, R), 0) // S
        ci_ = lax.broadcasted_iota(jnp.int32, (R, R), 1) // S
        mask = ri == ci_

        def Q(br, t, ci, h0=0, nh=G):
            q = jnp.dot(x_s[br, pl.ds(ci * MC, MC), :], wq_s[t, :, h0 * DH:(h0 + nh) * DH], preferred_element_type=F32).astype(BF)
            return [q[:, h * DH:(h + 1) * DH] for h in range(nh)]
        def QK(t, ci, qh_list):
            e_ = {}
            for h in range(G):
                for p in range(NPC):
                    qh = qh_list[h][p * R:(p + 1) * R, :]
                    b0 = ci * RB + p * PB
                    kk = k_s[t, b0:b0 + PB, h].reshape(R, DH)
                    s = lax.dot_general(qh, kk, NT_DIMS, preferred_element_type=F32)
                    s = jnp.where(mask, s, -jnp.inf)
                    m = jnp.max(s, axis=-1, keepdims=True)
                    e = jnp.exp2((s - m) * c)
                    l = jnp.sum(e, axis=-1, keepdims=True)
                    e_[(p, h)] = (e.astype(BF), l)
            return e_
        def PV(t, ci, e_):
            rows = []
            for p in range(NPC):
                cols = []
                for h in range(G):
                    b0 = ci * RB + p * PB
                    vv = v_s[t, b0:b0 + PB, h].reshape(R, DH)
                    eb, l = e_[(p, h)]
                    o = jnp.dot(eb, vv, preferred_element_type=F32)
                    cols.append((o * pl.reciprocal(l, approx=True)).astype(BF))
                rows.append(jnp.concatenate(cols, axis=1) if G > 1 else cols[0])
            return jnp.concatenate(rows, axis=0)
        def O(br, g, t, ci, o):
            static = isinstance(t, int)
            for s_ in range(OSUB):
                oi = ci * OSUB + s_
                rs = pl.ds(oi * MO, MO)
                new = jnp.dot(o[s_ * MO:(s_ + 1) * MO], wo_s[t], preferred_element_type=F32)
                if static:
                    if g > 0: new = new + acc[br, rs, :]
                    acc[br, rs, :] = new
                else:
                    new = new + jnp.where(g == 0, 0.0, acc[br, rs, :])
                    acc[br, rs, :] = new
                    out_s[br, rs, :] = new.astype(BF)
                    for b_ in range(2):
                        @pl.when(t == b_ * NG + NG - 1)
                        def _():
                            out_dma(b_, oi).start()

        def attn_o(br, g, t, qs, more_q=None):
            e = QK(t, 0, qs[0])
            for ci in range(NC):
                if ci + 1 < NC and more_q is not None:
                    qs[ci + 1] = more_q(ci + 1)
                if more_q is None and ci + 1 < NC:
                    e_next = QK(t, ci + 1, qs[ci + 1])
                    o = PV(t, ci, e)
                    e = e_next
                else:
                    o = PV(t, ci, e)
                    if ci + 1 < NC:
                        e = QK(t, ci + 1, qs[ci + 1])
                O(br, g, t, ci, o)

        qc = {t: {ci: [None] * G for ci in range(NC)} for t in range(CS)}
        def coldQ(piece, ci):
            t, h0, nh = piece
            qc[t][ci][h0:h0 + nh] = Q(0, t, ci, h0, nh)
        for d in cold_dmas[0]: d.wait()
        coldQ(pieces[0], 0)
        for d in cold_dmas[1]: d.wait()
        coldQ(pieces[0], 1); coldQ(pieces[0], 2)
        for d in cold_dmas[2]: d.wait()
        coldQ(pieces[0], 3)
        if len(pieces) > 1:
            for ci in range(NC): coldQ(pieces[1], ci)
        if len(pieces) > 2:
            for d in cold_dmas[3]: d.wait()
            for p_ in pieces[2:]:
                for ci in range(NC): coldQ(p_, ci)
        for t in range(CS):
            for d in step_dmas(t, False): d.wait()
            attn_o(0, t, t, qc[t])

        def body(t, carry):
            br = t // NG
            g = t % NG
            for d in step_dmas(t, True): d.wait()
            @pl.when(t == NG)
            def _():
                x_dma(1, 0, M, SEM_XB).wait()
            qs = {0: Q(br, t, 0)}
            attn_o(br, g, t, qs, more_q=lambda ci: Q(br, t, ci))
            return carry
        lax.fori_loop(CS, NT, body, 0)
        for b_ in range(2):
            for oi in range(NO):
                out_dma(b_, oi).wait()

    def fn(A_x, A_k, A_v, A_wq, A_wo, B_x, B_k, B_v, B_wq, B_wo):
        anyspec = pl.BlockSpec(memory_space=pl.ANY)
        out = pl.pallas_call(
            kernel,
            in_specs=[anyspec] * 10,
            out_specs=anyspec,
            out_shape=jax.ShapeDtypeStruct((M, 2 * D), BF),
            scratch_shapes=[
                pltpu.VMEM((2, M, D), BF),
                pltpu.VMEM((NT, B, G, S, DH), BF),
                pltpu.VMEM((NT, B, G, S, DH), BF),
                pltpu.VMEM((NT, D, GW), BF),
                pltpu.VMEM((NT, GW, D), BF),
                pltpu.VMEM((2, M, D), F32),
                pltpu.VMEM((2, M, D), BF),
                pltpu.SemaphoreType.DMA((NT + 3 + 4,)),
            ],
            compiler_params=pltpu.CompilerParams(vmem_limit_bytes=120 * 1024 * 1024,
                                                 disable_bounds_checks=nobc,
                                                 disable_semaphore_checks=nosc),
        )(A_x.reshape(M, D), A_k, A_v, A_wq, A_wo, B_x.reshape(M, D), B_k, B_v, B_wq, B_wo)
        return out.reshape(B, S, 2 * D)
    return fn


_FN = build(G=4, CS=2, OSUB=4)


@jax.jit
def pallas_concat_heads__gqa_block_cached__gqa_block_cached__near_ridge_kernel(
    A_x, A_k_cache, A_v_cache, A_wq, A_wo, B_x, B_k_cache, B_v_cache, B_wq, B_wo
):
    return _FN(A_x, A_k_cache, A_v_cache, A_wq, A_wo, B_x, B_k_cache, B_v_cache, B_wq, B_wo)
```

```python
import math

import jax
import jax.numpy as jnp
from jax import lax
import jax.experimental.pallas as pl
import jax.experimental.pallas.tpu as pltpu

F32 = jnp.float32
BF = jnp.bfloat16
_NT = (((1,), (1,)), ((), ()))

_SA = [[((0, 0), 1), ((1, 1), 1)], [((1, 0), 1), ((1, 1), 1)], [((0, 0), 1)], [((1, 1), 1)],
       [((0, 0), 1), ((0, 1), 1)], [((1, 0), 1), ((0, 0), -1)], [((0, 1), 1), ((1, 1), -1)]]
_SB = [[((0, 0), 1), ((1, 1), 1)], [((0, 0), 1)], [((0, 1), 1), ((1, 1), -1)], [((1, 0), 1), ((0, 0), -1)],
       [((1, 1), 1)], [((0, 0), 1), ((0, 1), 1)], [((1, 0), 1), ((1, 1), 1)]]
_SC = {(0, 0): [(0, 1), (3, 1), (4, -1), (6, 1)], (0, 1): [(2, 1), (4, 1)],
       (1, 0): [(1, 1), (3, 1)], (1, 1): [(0, 1), (1, -1), (2, 1), (5, 1)]}
_ORDER = [2, 4, 0, 3, 6, 1, 5]


def _kron(outer, inner):
    return [((o[0] * 2 + i[0], o[1] * 2 + i[1]), so * si) for (o, so) in outer for (i, si) in inner]


def _lhs_terms(p):
    t = _kron(_SA[p // 7], _SA[p % 7])
    return [t[0], t[3], t[1], t[2]] if len(t) == 4 else t


def _signed_sum(get, terms):
    acc = get(terms[0][0])
    assert terms[0][1] > 0
    for idx, sgn in terms[1:]:
        acc = acc + get(idx) if sgn > 0 else acc - get(idx)
    return acc


def build(EQ=True, NEWTON=False, GO=3, LAG=4, FR=192, QC=4, FSP=3, CSP=2, NG=21, TSKIP=1,
          STAGES=((192, 2), (384, 2), (528, 3), (768, 5))):
    B, S, D, H, DH = 32, 48, 512, 32, 128
    M = B * S
    GQ, SW, GA, HQ = 8, 4, 16, 8
    NQ, NS, NA, NHQ, NSL = H // GQ, GQ // SW, H // GA, GA // HQ, H // HQ
    R = 2 * S
    NB, NP = 4, 49
    NC = M // (NB * R)
    KB, NW = HQ * DH // NB, D // NB
    HPB = HQ // NB
    TT = 16
    NTU, TPI, UPS = 2 * NSL, 3, 2
    QR = M - FR
    stages = tuple(STAGES) + ((QR, GQ),)
    cexp = (DH ** -0.5) * math.log2(math.e)
    porder = [o * 7 + i for o in _ORDER for i in _ORDER]
    SEM_Q, SEM_A = 0, 2 * NQ
    SEM_COLD = SEM_A + 2 * NA
    NSEM = SEM_COLD + len(stages) - 1

    def new_slabs(n):
        need = lambda m: {min(u, NTU - 1) // UPS for u in range(TPI * m, TPI * m + TPI)}
        return sorted(need(n) - set().union(*[need(m) for m in range(n)]))

    def kernel(ax, ak, av, awq, awo, bx, bk, bv, bwq, bwo, out_hbm,
               x_s, k_s, v_s, wq_s, wo_s, q_s, t_s, d_s, m_s, c_s, p_s, out_s, sems):
        src = ((ax, ak, av, awq, awo), (bx, bk, bv, bwq, bwo))
        st = lambda i: i if isinstance(i, int) else 0

        def x_dma(br, lo, n, sem):
            return pltpu.make_async_copy(src[br][0].at[pl.ds(lo, n)], x_s.at[br, pl.ds(lo, n)], sems.at[sem])

        def wq_dmas(br, j, sem, h0=0, h1=GQ):
            out = []
            while h0 < h1:
                e = min(h1, (h0 // SW + 1) * SW)
                out.append(pltpu.make_async_copy(
                    src[st(br)][3].at[:, pl.ds((st(j) * GQ + h0) * DH, (e - h0) * DH)],
                    wq_s.at[(br * NQ + j) * NS + h0 // SW, :, pl.ds((h0 % SW) * DH, (e - h0) * DH)],
                    sems.at[sem]))
                h0 = e
            return out

        def wo_dmas(br, sl, sem):
            rows = pl.ds(sl * HQ * DH, HQ * DH)
            if sl // NHQ == 0:
                return [pltpu.make_async_copy(src[st(br)][4].at[rows, :], wo_s.at[br * NSL + sl], sems.at[sem])]
            return [pltpu.make_async_copy(src[st(br)][4].at[rows, pl.ds((NB - 1 - nb) * NW, NW)],
                                          wo_s.at[br * NSL + sl, :, pl.ds(nb * NW, NW)], sems.at[sem])
                    for nb in range(NB)]

        def kv_dmas(br, j):
            t = br * NA + j
            hs = pl.ds(st(j) * GA, GA)
            return [pltpu.make_async_copy(src[st(br)][1].at[:, hs], k_s.at[t], sems.at[SEM_A + t]),
                    pltpu.make_async_copy(src[st(br)][2].at[:, hs], v_s.at[t], sems.at[SEM_A + t])]

        def out_dma(br, blk):
            rows = pl.ds(blk * R, R)
            return pltpu.make_async_copy(out_s.at[br, rows], out_hbm.at[rows, pl.ds(br * D, D)],
                                         sems.at[SEM_Q + br])

        cold = []
        pr, ph = 0, 0
        for si, (r, h) in enumerate(stages):
            sem = SEM_Q if si == 0 else SEM_COLD + si - 1
            r = M if si == len(stages) - 1 else r
            cold.append(wq_dmas(0, 0, sem, ph, h) + ([x_dma(0, pr, r - pr, sem)] if r > pr else []))
            pr, ph = r, h
        for grp in cold:
            for d in grp:
                d.start()
        for br in range(2):
            if br == 1:
                x_dma(1, 0, M, SEM_Q + NQ).start(priority=1)
            for j in range(1 - br, NQ):
                sem = SEM_Q + br * NQ + j
                dmas = wq_dmas(br, j, sem)
                for sl in new_slabs(j - (1 - br)):
                    dmas += wo_dmas(br, sl, sem)
                for d in dmas:
                    d.start(priority=1)
            for j in range(NA):
                for d in kv_dmas(br, j):
                    d.start(priority=1)

        row = lax.broadcasted_iota(jnp.int32, (R, DH), 0)
        col = lax.broadcasted_iota(jnp.int32, (R, DH), 1)
        mask = (row // S) == (col // S)

        def recip(v, newton):
            r_ = pl.reciprocal(v, approx=True)
            return r_ * (2.0 - v * r_) if newton else r_

        def q_proj(br, j, r0, r1, h0, h1):
            while h0 < h1:
                e = min(h1, (h0 // SW + 1) * SW)
                w = wq_s[(br * NQ + j) * NS + h0 // SW, :, (h0 % SW) * DH:(h0 % SW + e - h0) * DH]
                q = jnp.dot(x_s[br, r0:r1, :], w, preferred_element_type=F32)
                for h in range(h0, e):
                    q_s[j * GQ + h, r0:r1, :] = q[:, (h - h0) * DH:(h - h0 + 1) * DH].astype(BF)
                h0 = e
            return q

        def t_tile(br, u, r0, gates, pred, dacc):
            sl, half = u >> 1, u & 1
            lo = pl.multiple_of(half * DH + r0, TT)
            w = {(kb, nb): wo_s[br * NSL + sl, pl.ds(kb * KB + lo, TT), nb * NW:(nb + 1) * NW].astype(F32)
                 for kb in range(NB) for nb in range(NB)}
            if EQ:
                diag = (lax.broadcasted_iota(jnp.int32, (TT, DH), 1)
                        == lax.broadcasted_iota(jnp.int32, (TT, DH), 0) + r0)
                for kb in range(NB):
                    a = [jnp.abs(w[(kb, nb)]) for nb in range(NB)]
                    d = jnp.sum((a[0] + a[1]) + (a[2] + a[3]), axis=-1, keepdims=True)
                    d = jnp.clip(d, 2.0 ** -100, 2.0 ** 100)
                    dinv = recip(d, True)
                    for nb in range(NB):
                        w[(kb, nb)] = w[(kb, nb)] * dinv
                    part = jnp.where(diag, d, 0.0)
                    dacc[kb] = part if r0 == 0 else dacc[kb] + part
                    if r0 + TT == DH:
                        drow = jnp.sum(jnp.where(pred, dacc[kb], gates[-1]), axis=0, keepdims=True)
                        d_s[sl * HQ + kb * HPB + half] = jnp.broadcast_to(drow, (8, DH))
            for o in range(7):
                ob = {ii: _signed_sum(lambda oi: w[(oi[0] * 2 + ii[0], oi[1] * 2 + ii[1])], _SB[o])
                      for ii in ((0, 0), (0, 1), (1, 0), (1, 1))}
                for i in range(7):
                    p = o * 7 + i
                    tv = _signed_sum(ob.get, _SB[i])
                    t_s[sl * NP + p, pl.ds(lo, TT), :] = jnp.where(pred, tv, gates[p * len(gates) // NP]).astype(BF)

        pr, ph = 0, 0
        for si, (r, h) in enumerate(stages):
            for d in cold[si]:
                d.wait()
            if r > pr and ph > 0:
                q_proj(0, 0, pr, r, 0, ph)
            if h > ph:
                q_proj(0, 0, 0, r, ph, h)
            pr, ph = r, h

        def q_body(j, br):
            sem = SEM_Q + br * NQ + j
            n = j - (1 - br)
            for d in wq_dmas(br, j, sem):
                d.wait()
            for n_ in range(NQ):
                if new_slabs(n_):
                    @pl.when(n == n_)
                    def _():
                        for sl in new_slabs(n_):
                            for d in wo_dmas(br, sl, sem):
                                d.wait()
            rc = QR // QC
            tiles = [(k, r0) for k in range(TPI) for r0 in range(0, DH, TT)]
            per = -(-len(tiles) // (NS * QC - TSKIP))
            slots = [(nt, r_) for nt in range(SW) for r_ in range(0, rc - TT + 1, TT)]
            pred = n >= 0
            dacc = {}
            for qi in range(NS * QC):
                h0, ri = (qi // QC) * SW, qi % QC
                q = q_proj(br, j, ri * rc, (ri + 1) * rc, h0, h0 + SW)
                mine = tiles[qi * per:(qi + 1) * per]
                for ti, (k, r0) in enumerate(mine):
                    gates = []
                    for gi in range(NG):
                        nt, r_ = slots[(ti * NG + gi) * len(slots) // (len(mine) * NG)]
                        gates.append(q[r_:r_ + TT, nt * DH:(nt + 1) * DH])
                    t_tile(br, jnp.minimum(n * TPI + k, NTU - 1), r0, gates, pred, dacc)
            return br

        def ao_body(j, br):
            t = br * NA + j
            for d in kv_dmas(br, j):
                d.wait()
            always = j >= 0
            zpad = jnp.zeros((DH - R, DH), BF)
            chunks = [(ci, hq) for ci in range(NC) for hq in range(NHQ)]
            units = [(ci * NB + p, hq * HQ + h) for (ci, hq) in chunks for p in range(NB) for h in range(HQ)]
            upc = NB * HQ
            soft, outs, hist = {}, {}, []
            pending, cqueue, cdone, ctick = [], [], set(), [0]

            def qk(u):
                p, h = units[u]
                kk = jnp.concatenate([k_s[t, 2 * p:2 * p + 2, h].reshape(R, DH), zpad], axis=0)
                s = lax.dot_general(q_s[j * GA + h, p * R:(p + 1) * R, :], kk, _NT, preferred_element_type=F32)
                s = jnp.where(mask, s, -jnp.inf)
                e = jnp.exp2((s - jnp.max(s, axis=-1, keepdims=True)) * cexp)
                soft[u] = (e, recip(jnp.sum(e, axis=-1, keepdims=True), NEWTON))

            def pv(u):
                p, h = units[u]
                vv = jnp.concatenate([v_s[t, 2 * p:2 * p + 2, h].reshape(R, DH), zpad], axis=0)
                e, r_ = soft.pop(u)
                if len(hist) >= GO:
                    e = jnp.where(always, e, hist[-GO])
                o = jnp.dot(e.astype(BF), vv, preferred_element_type=F32) * r_
                if EQ:
                    o = o * d_s[j * GA + h, 0:1, :]
                hist.append(o)
                outs[(p, h)] = o

            def recombine(ci, rb, nb, terms, first, last, gate):
                rows = pl.ds((ci * NB + rb) * R, R)
                if first:
                    cv = jnp.where(j == 0, 0.0, c_s[0, NB - 1 - nb, rows, :])
                else:
                    cv = p_s[nb, pl.ds(rb * R, R), :]
                if gate is not None:
                    cv = jnp.where(always, cv, gate)
                for p, sgn in terms:
                    mv = m_s[p, pl.ds((ci % 2) * R, R), :]
                    cv = cv + mv if sgn > 0 else cv - mv
                if not last:
                    p_s[nb, pl.ds(rb * R, R), :] = cv
                    return
                c_s[j, nb, rows, :] = cv
                out_s[br, rows, (NB - 1 - nb) * NW:(NB - nb) * NW] = cv.astype(BF)
                cdone.add((ci, rb, nb))
                if all((ci, rb, n_) in cdone for n_ in range(NB)):
                    for b_ in range(2):
                        @pl.when(t == b_ * NA + NA - 1)
                        def _():
                            out_dma(b_, ci * NB + rb).start()

            def product(u, p):
                ci, hq = chunks[u]
                blk = lambda idx: jnp.concatenate(
                    [outs[(ci * NB + idx[0], hq * HQ + idx[1] * HPB + h)] for h in range(HPB)], axis=1)
                a = _signed_sum(blk, _lhs_terms(p)).astype(BF)
                mv = jnp.dot(a, t_s[(j * NHQ + hq) * NP + p], preferred_element_type=F32)
                ctick[0] += 1
                if cqueue and (ctick[0] >= CSP or u == len(chunks) - 1):
                    ctick[0] = 0
                    recombine(*cqueue.pop(0), mv)
                assert all(task[0] >= ci - 1 for task in cqueue)
                rs = pl.ds((ci % 2) * R, R)
                if hq > 0:
                    mv = mv + m_s[p, rs, :]
                m_s[p, rs, :] = mv
                if hq < NHQ - 1:
                    return
                o_, i_ = divmod(p, 7)
                for oblk, oterms in _SC.items():
                    oseq = sorted(oterms, key=lambda x: _ORDER.index(x[0]))
                    for pos, (ko, so) in enumerate(oseq):
                        if ko != o_:
                            continue
                        for iblk, iterms in _SC.items():
                            iseq = sorted(iterms, key=lambda x: _ORDER.index(x[0]))
                            if iseq[-1][0] == i_:
                                cqueue.append((ci, oblk[0] * 2 + iblk[0], oblk[1] * 2 + iblk[1],
                                               [(o_ * 7 + ki, so * si) for ki, si in iseq],
                                               pos == 0, pos == len(oseq) - 1))

            fill = list(range(GA)) if FR else []
            tick = [0]

            def filler():
                if fill and tick[0] % FSP == 0:
                    h = fill.pop(0)
                    q_proj(br, j * (GA // GQ) + h // GQ, QR, M, h % GQ, h % GQ + 1)
                tick[0] += 1

            for u in range(LAG):
                filler()
                qk(u)
            credit = 0.0
            for u in range(len(units)):
                filler()
                pv(u)
                if u + LAG < len(units):
                    assert not fill or units[u + LAG][0] * R + R <= QR
                    qk(u + LAG)
                if (u + 1) % upc == 0:
                    pending += [(u // upc, p) for p in porder]
                credit += NP / upc
                n = int(credit + 1e-9)
                credit -= n
                for _ in range(min(n, len(pending))):
                    product(*pending.pop(0))
            while pending:
                product(*pending.pop(0))
            while cqueue:
                recombine(*cqueue.pop(0), None)
            return br

        def branch(br, carry):
            @pl.when(br == 1)
            def _():
                x_dma(1, 0, M, SEM_Q + NQ).wait()
            lax.fori_loop(1 - br, NQ, q_body, br)
            lax.fori_loop(0, NA, ao_body, br)
            return carry

        lax.fori_loop(0, 2, branch, 0)
        for b_ in range(2):
            for blk in range(M // R):
                out_dma(b_, blk).wait()

    def fn(A_x, A_k, A_v, A_wq, A_wo, B_x, B_k, B_v, B_wq, B_wo):
        anyspec = pl.BlockSpec(memory_space=pl.ANY)
        out = pl.pallas_call(
            kernel,
            in_specs=[anyspec] * 10,
            out_specs=anyspec,
            out_shape=jax.ShapeDtypeStruct((M, 2 * D), BF),
            scratch_shapes=[
                pltpu.VMEM((2, M, D), BF),
                pltpu.VMEM((2 * NA, B, GA, S, DH), BF),
                pltpu.VMEM((2 * NA, B, GA, S, DH), BF),
                pltpu.VMEM((2 * NQ * NS, D, SW * DH), BF),
                pltpu.VMEM((2 * NSL, HQ * DH, D), BF),
                pltpu.VMEM((H, M, DH), BF),
                pltpu.VMEM((NSL * NP, KB, NW), BF),
                pltpu.VMEM((H, 8, DH), F32),
                pltpu.VMEM((NP, 2 * R, NW), F32),
                pltpu.VMEM((NA, NB, M, NW), F32),
                pltpu.VMEM((NB, NB * R, NW), F32),
                pltpu.VMEM((2, M, D), BF),
                pltpu.SemaphoreType.DMA((NSEM,)),
            ],
            compiler_params=pltpu.CompilerParams(vmem_limit_bytes=120 * 1024 * 1024),
        )(A_x.reshape(M, D), A_k, A_v, A_wq, A_wo, B_x.reshape(M, D), B_k, B_v, B_wq, B_wo)
        return out.reshape(B, S, 2 * D)
    return fn


_FN = build()


@jax.jit
def pallas_concat_heads__gqa_block_cached__gqa_block_cached__near_ridge_kernel(
    A_x, A_k_cache, A_v_cache, A_wq, A_wo, B_x, B_k_cache, B_v_cache, B_wq, B_wo
):
    return _FN(A_x, A_k_cache, A_v_cache, A_wq, A_wo, B_x, B_k_cache, B_v_cache, B_wq, B_wo)
```

```python
import math

import jax
import jax.numpy as jnp
from jax import lax
import jax.experimental.pallas as pl
import jax.experimental.pallas.tpu as pltpu

F32 = jnp.float32
BF = jnp.bfloat16
_NT = (((1,), (1,)), ((), ()))

_SA = [[((0, 0), 1), ((1, 1), 1)], [((1, 0), 1), ((1, 1), 1)], [((0, 0), 1)], [((1, 1), 1)],
       [((0, 0), 1), ((0, 1), 1)], [((1, 0), 1), ((0, 0), -1)], [((0, 1), 1), ((1, 1), -1)]]
_SB = [[((0, 0), 1), ((1, 1), 1)], [((0, 0), 1)], [((0, 1), 1), ((1, 1), -1)], [((1, 0), 1), ((0, 0), -1)],
       [((1, 1), 1)], [((0, 0), 1), ((0, 1), 1)], [((1, 0), 1), ((1, 1), 1)]]
_SC = {(0, 0): [(0, 1), (3, 1), (4, -1), (6, 1)], (0, 1): [(2, 1), (4, 1)],
       (1, 0): [(1, 1), (3, 1)], (1, 1): [(0, 1), (1, -1), (2, 1), (5, 1)]}
_ORDER = [2, 4, 0, 3, 6, 1, 5]


def _lhs_terms(p):
    t = [((o[0] * 2 + i[0], o[1] * 2 + i[1]), so * si)
         for (o, so) in _SA[p // 7] for (i, si) in _SA[p % 7]]
    return [t[0], t[3], t[1], t[2]] if len(t) == 4 else t


def _signed_sum(get, terms):
    assert terms[0][1] > 0
    acc = get(terms[0][0])
    for idx, sgn in terms[1:]:
        acc = acc + get(idx) if sgn > 0 else acc - get(idx)
    return acc


@jax.jit
def pallas_concat_heads__gqa_block_cached__gqa_block_cached__near_ridge_kernel(
    A_x: jax.Array,
    A_k_cache: jax.Array,
    A_v_cache: jax.Array,
    A_wq: jax.Array,
    A_wo: jax.Array,
    B_x: jax.Array,
    B_k_cache: jax.Array,
    B_v_cache: jax.Array,
    B_wq: jax.Array,
    B_wo: jax.Array,
):
    B, S, D = A_x.shape
    _, H, SK, DH = A_k_cache.shape
    assert (B, S, D, H, SK, DH) == (32, 48, 512, 32, 48, 128) and A_wq.shape == (D, H * DH)
    M = B * S
    R = 2 * S
    GQ, SW = 8, 4
    GA, HQ = 16, 8
    NQ, NS, NA, NHQ, NSL = H // GQ, GQ // SW, H // GA, GA // HQ, H // HQ
    NB, NP = 4, 49
    NC = M // (NB * R)
    KB, NW, HPB = HQ * DH // NB, D // NB, HQ // NB
    TT = 16
    NTU, TPI = 2 * NSL, 3
    FR = 192
    QR = M - FR
    QC = 4
    STAGES = ((192, 2), (384, 2), (528, 3), (768, 5), (QR, GQ))
    LAG, GO, FSP, CSP, NG = 4, 3, 3, 2, 21
    cexp = (DH ** -0.5) * math.log2(math.e)
    porder = [o * 7 + i for o in _ORDER for i in _ORDER]
    SEM_Q, SEM_A = 0, 2 * NQ
    SEM_COLD = SEM_A + 2 * NA
    NSEM = SEM_COLD + len(STAGES) - 1

    def new_slabs(n):
        need = lambda m: {min(u, NTU - 1) // 2 for u in range(TPI * m, TPI * m + TPI)}
        return sorted(need(n) - set().union(*[need(m) for m in range(n)]))

    def kernel(ax, ak, av, awq, awo, bx, bk, bv, bwq, bwo, out_hbm,
               x_s, k_s, v_s, wq_s, wo_s, q_s, t_s, d_s, m_s, c_s, p_s, out_s, sems):
        src = ((ax, ak, av, awq, awo), (bx, bk, bv, bwq, bwo))
        st = lambda i: i if isinstance(i, int) else 0

        def x_dma(br, lo, n, sem):
            return pltpu.make_async_copy(src[br][0].at[pl.ds(lo, n)], x_s.at[br, pl.ds(lo, n)],
                                         sems.at[sem])

        def wq_dmas(br, j, sem, h0=0, h1=GQ):
            out = []
            while h0 < h1:
                e = min(h1, (h0 // SW + 1) * SW)
                out.append(pltpu.make_async_copy(
                    src[st(br)][3].at[:, pl.ds((st(j) * GQ + h0) * DH, (e - h0) * DH)],
                    wq_s.at[(br * NQ + j) * NS + h0 // SW, :, pl.ds((h0 % SW) * DH, (e - h0) * DH)],
                    sems.at[sem]))
                h0 = e
            return out

        def wo_dmas(br, sl, sem):
            rows = pl.ds(sl * HQ * DH, HQ * DH)
            if sl // NHQ == 0:
                return [pltpu.make_async_copy(src[st(br)][4].at[rows, :], wo_s.at[br * NSL + sl],
                                              sems.at[sem])]
            return [pltpu.make_async_copy(src[st(br)][4].at[rows, pl.ds((NB - 1 - nb) * NW, NW)],
                                          wo_s.at[br * NSL + sl, :, pl.ds(nb * NW, NW)], sems.at[sem])
                    for nb in range(NB)]

        def kv_dmas(br, j):
            t = br * NA + j
            hs = pl.ds(st(j) * GA, GA)
            return [pltpu.make_async_copy(src[st(br)][1].at[:, hs], k_s.at[t], sems.at[SEM_A + t]),
                    pltpu.make_async_copy(src[st(br)][2].at[:, hs], v_s.at[t], sems.at[SEM_A + t])]

        def out_dma(br, blk, c0=0, nc=D):
            rows = pl.ds(blk * R, R)
            return pltpu.make_async_copy(out_s.at[br, rows, pl.ds(c0, nc)],
                                         out_hbm.at[rows, pl.ds(br * D + c0, nc)], sems.at[SEM_Q + br])

        cold = []
        pr, ph = 0, 0
        for si, (r, h) in enumerate(STAGES):
            sem = SEM_Q if si == 0 else SEM_COLD + si - 1
            r = M if si == len(STAGES) - 1 else r
            cold.append(wq_dmas(0, 0, sem, ph, h) + [x_dma(0, pr, r - pr, sem)])
            pr, ph = r, h
        for grp in cold:
            for d in grp:
                d.start()
        for br in range(2):
            if br == 1:
                x_dma(1, 0, M, SEM_Q + NQ).start(priority=1)
            for j in range(1 - br, NQ):
                sem = SEM_Q + br * NQ + j
                dmas = wq_dmas(br, j, sem)
                for sl in new_slabs(j - (1 - br)):
                    dmas += wo_dmas(br, sl, sem)
                for d in dmas:
                    d.start(priority=1)
            for j in range(NA):
                for d in kv_dmas(br, j):
                    d.start(priority=1)

        mask = (lax.broadcasted_iota(jnp.int32, (R, DH), 0) // S
                == lax.broadcasted_iota(jnp.int32, (R, DH), 1) // S)

        def q_proj(br, j, r0, r1, h0, h1):
            while h0 < h1:
                e = min(h1, (h0 // SW + 1) * SW)
                w = wq_s[(br * NQ + j) * NS + h0 // SW, :, (h0 % SW) * DH:(h0 % SW + e - h0) * DH]
                q = jnp.dot(x_s[br, r0:r1, :], w, preferred_element_type=F32)
                for h in range(h0, e):
                    q_s[j * GQ + h, r0:r1, :] = q[:, (h - h0) * DH:(h - h0 + 1) * DH].astype(BF)
                h0 = e
            return q

        def t_tile(br, u, r0, gates, always, dacc):
            sl, half = u >> 1, u & 1
            lo = pl.multiple_of(half * DH + r0, TT)
            w = {(kb, nb): wo_s[br * NSL + sl, pl.ds(kb * KB + lo, TT), nb * NW:(nb + 1) * NW].astype(F32)
                 for kb in range(NB) for nb in range(NB)}
            diag = (lax.broadcasted_iota(jnp.int32, (TT, DH), 1)
                    == lax.broadcasted_iota(jnp.int32, (TT, DH), 0) + r0)
            for kb in range(NB):
                a = [jnp.abs(w[(kb, nb)]) for nb in range(NB)]
                d = jnp.sum((a[0] + a[1]) + (a[2] + a[3]), axis=-1, keepdims=True)
                d = jnp.clip(d, 2.0 ** -100, 2.0 ** 100)
                dinv = pl.reciprocal(d, approx=True)
                dinv = dinv * (2.0 - d * dinv)
                for nb in range(NB):
                    w[(kb, nb)] = w[(kb, nb)] * dinv
                part = jnp.where(diag, d, 0.0)
                dacc[kb] = part if r0 == 0 else dacc[kb] + part
                if r0 + TT == DH:
                    drow = jnp.sum(jnp.where(always, dacc[kb], gates[-1]), axis=0, keepdims=True)
                    d_s[sl * HQ + kb * HPB + half] = jnp.broadcast_to(drow, (8, DH))
            for o in range(7):
                ob = {ii: _signed_sum(lambda oi: w[(oi[0] * 2 + ii[0], oi[1] * 2 + ii[1])], _SB[o])
                      for ii in ((0, 0), (0, 1), (1, 0), (1, 1))}
                for i in range(7):
                    p = o * 7 + i
                    tv = jnp.where(always, _signed_sum(ob.get, _SB[i]), gates[p * len(gates) // NP])
                    t_s[sl * NP + p, pl.ds(lo, TT), :] = tv.astype(BF)

        pr, ph = 0, 0
        for si, (r, h) in enumerate(STAGES):
            for d in cold[si]:
                d.wait()
            if ph > 0:
                q_proj(0, 0, pr, r, 0, ph)
            if h > ph:
                q_proj(0, 0, 0, r, ph, h)
            pr, ph = r, h

        def q_body(j, br):
            sem = SEM_Q + br * NQ + j
            n = j - (1 - br)
            for d in wq_dmas(br, j, sem):
                d.wait()
            for n_ in range(NQ):
                if new_slabs(n_):
                    @pl.when(n == n_)
                    def _():
                        for sl in new_slabs(n_):
                            for d in wo_dmas(br, sl, sem):
                                d.wait()
            rc = QR // QC
            tiles = [(k, r0) for k in range(TPI) for r0 in range(0, DH, TT)]
            per = len(tiles) // (NS * QC)
            slots = [(nt, r_) for nt in range(SW) for r_ in range(0, rc - TT + 1, TT)]
            always = n >= 0
            dacc = {}
            for qi in range(NS * QC):
                h0, ri = (qi // QC) * SW, qi % QC
                q = q_proj(br, j, ri * rc, (ri + 1) * rc, h0, h0 + SW)
                for ti, (k, r0) in enumerate(tiles[qi * per:(qi + 1) * per]):
                    gates = []
                    for gi in range(NG):
                        nt, r_ = slots[(ti * NG + gi) * len(slots) // (per * NG)]
                        gates.append(q[r_:r_ + TT, nt * DH:(nt + 1) * DH])
                    t_tile(br, jnp.minimum(n * TPI + k, NTU - 1), r0, gates, always, dacc)
            return br

        def ao_body(j, br):
            t = br * NA + j
            for d in kv_dmas(br, j):
                d.wait()
            always = j >= 0
            zpad = jnp.zeros((DH - R, DH), BF)
            chunks = [(ci, hq) for ci in range(NC) for hq in range(NHQ)]
            units = [(ci * NB + p, hq * HQ + h)
                     for (ci, hq) in chunks for p in range(NB) for h in range(HQ)]
            upc = NB * HQ
            soft, outs, hist, lastm = {}, {}, [], {}
            pending, cqueue, cdone, ctick = [], [], set(), [0]

            def qk(u):
                p, h = units[u]
                kk = jnp.concatenate([k_s[t, 2 * p:2 * p + 2, h].reshape(R, DH), zpad], axis=0)
                s = lax.dot_general(q_s[j * GA + h, p * R:(p + 1) * R, :], kk, _NT,
                                    preferred_element_type=F32)
                s = jnp.where(mask, s, -jnp.inf)
                e = jnp.exp2((s - jnp.max(s, axis=-1, keepdims=True)) * cexp)
                soft[u] = (e, pl.reciprocal(jnp.sum(e, axis=-1, keepdims=True), approx=True))

            def pv(u):
                p, h = units[u]
                vv = jnp.concatenate([v_s[t, 2 * p:2 * p + 2, h].reshape(R, DH), zpad], axis=0)
                e, rinv = soft.pop(u)
                if len(hist) >= GO:
                    e = jnp.where(always, e, hist[-GO])
                o = jnp.dot(e.astype(BF), vv, preferred_element_type=F32) * rinv
                o = o * d_s[j * GA + h, 0:1, :]
                hist.append(o)
                outs[(p, h)] = o

            def recombine(ci, rb, nb, terms, first, last, gate):
                blk = ci * NB + rb
                rows = pl.ds(blk * R, R)
                if first:
                    cv = jnp.where(j == 0, 0.0, c_s[0, NB - 1 - nb, rows, :])
                else:
                    cv = p_s[nb, pl.ds(rb * R, R), :]
                if gate is not None:
                    cv = jnp.where(always, cv, gate)
                for p, sgn in terms:
                    mv = lastm[p] if p in lastm else m_s[p, pl.ds((ci % 2) * R, R), :]
                    cv = cv + mv if sgn > 0 else cv - mv
                if not last:
                    p_s[nb, pl.ds(rb * R, R), :] = cv
                    return
                c_s[j, nb, rows, :] = cv
                out_s[br, rows, (NB - 1 - nb) * NW:(NB - nb) * NW] = cv.astype(BF)
                cdone.add((ci, rb, nb))
                fine = blk == M // R - 1
                if fine or all((ci, rb, n_) in cdone for n_ in range(NB)):
                    for b_ in range(2):
                        @pl.when(t == b_ * NA + NA - 1)
                        def _():
                            if fine:
                                out_dma(b_, blk, (NB - 1 - nb) * NW, NW).start()
                            else:
                                out_dma(b_, blk).start()

            def product(u, p):
                ci, hq = chunks[u]
                last_chunk = u == len(chunks) - 1
                blk = lambda idx: jnp.concatenate(
                    [outs[(ci * NB + idx[0], hq * HQ + idx[1] * HPB + h)] for h in range(HPB)], axis=1)
                a = _signed_sum(blk, _lhs_terms(p)).astype(BF)
                mv = jnp.dot(a, t_s[(j * NHQ + hq) * NP + p], preferred_element_type=F32)
                ctick[0] += 1
                if cqueue and (ctick[0] >= CSP or last_chunk):
                    ctick[0] = 0
                    recombine(*cqueue.pop(0), mv)
                assert all(task[0] >= ci - 1 for task in cqueue)
                rs = pl.ds((ci % 2) * R, R)
                if hq > 0:
                    mv = mv + m_s[p, rs, :]
                if last_chunk and p in porder[-2:]:
                    assert all(task[0] == ci for task in cqueue)
                    lastm[p] = mv
                else:
                    m_s[p, rs, :] = mv
                if hq < NHQ - 1:
                    return
                o_, i_ = divmod(p, 7)
                for oblk, oterms in _SC.items():
                    oseq = sorted(oterms, key=lambda x: _ORDER.index(x[0]))
                    for pos, (ko, so) in enumerate(oseq):
                        if ko != o_:
                            continue
                        for iblk, iterms in _SC.items():
                            iseq = sorted(iterms, key=lambda x: _ORDER.index(x[0]))
                            if iseq[-1][0] == i_:
                                cqueue.append((ci, oblk[0] * 2 + iblk[0], oblk[1] * 2 + iblk[1],
                                               [(o_ * 7 + ki, so * si) for ki, si in iseq],
                                               pos == 0, pos == len(oseq) - 1))

            fill = list(range(GA))
            tick = [0]

            def filler():
                if fill and tick[0] % FSP == 0:
                    h = fill.pop(0)
                    q_proj(br, j * (GA // GQ) + h // GQ, QR, M, h % GQ, h % GQ + 1)
                tick[0] += 1

            for u in range(LAG):
                filler()
                qk(u)
            credit = 0.0
            for u in range(len(units)):
                filler()
                pv(u)
                if u + LAG < len(units):
                    assert not fill or (units[u + LAG][0] + 1) * R <= QR
                    qk(u + LAG)
                if (u + 1) % upc == 0:
                    pending += [(u // upc, p) for p in porder]
                credit += NP / upc
                n = int(credit + 1e-9)
                credit -= n
                for _ in range(min(n, len(pending))):
                    product(*pending.pop(0))
            while pending:
                product(*pending.pop(0))
            while cqueue:
                recombine(*cqueue.pop(0), None)
            return br

        def branch(br, carry):
            @pl.when(br == 1)
            def _():
                x_dma(1, 0, M, SEM_Q + NQ).wait()
            lax.fori_loop(1 - br, NQ, q_body, br)
            lax.fori_loop(0, NA, ao_body, br)
            return carry

        lax.fori_loop(0, 2, branch, 0)
        for b_ in range(2):
            for blk in range(M // R - 1):
                out_dma(b_, blk).wait()
            for nb in range(NB):
                out_dma(b_, M // R - 1, nb * NW, NW).wait()

    anyspec = pl.BlockSpec(memory_space=pl.ANY)
    out = pl.pallas_call(
        kernel,
        in_specs=[anyspec] * 10,
        out_specs=anyspec,
        out_shape=jax.ShapeDtypeStruct((M, 2 * D), BF),
        scratch_shapes=[
            pltpu.VMEM((2, M, D), BF),
            pltpu.VMEM((2 * NA, B, GA, S, DH), BF),
            pltpu.VMEM((2 * NA, B, GA, S, DH), BF),
            pltpu.VMEM((2 * NQ * NS, D, SW * DH), BF),
            pltpu.VMEM((2 * NSL, HQ * DH, D), BF),
            pltpu.VMEM((H, M, DH), BF),
            pltpu.VMEM((NSL * NP, KB, NW), BF),
            pltpu.VMEM((H, 8, DH), F32),
            pltpu.VMEM((NP, 2 * R, NW), F32),
            pltpu.VMEM((NA, NB, M, NW), F32),
            pltpu.VMEM((NB, NB * R, NW), F32),
            pltpu.VMEM((2, M, D), BF),
            pltpu.SemaphoreType.DMA((NSEM,)),
        ],
        compiler_params=pltpu.CompilerParams(vmem_limit_bytes=120 * 1024 * 1024),
    )(A_x.reshape(M, D), A_k_cache, A_v_cache, A_wq, A_wo,
      B_x.reshape(M, D), B_k_cache, B_v_cache, B_wq, B_wo)
    return out.reshape(B, S, 2 * D)
```

```python
import math

import jax
import jax.numpy as jnp
from jax import lax
import jax.experimental.pallas as pl
import jax.experimental.pallas.tpu as pltpu

F32 = jnp.float32
BF = jnp.bfloat16
_NT = (((1,), (1,)), ((), ()))

_SA = [[((0, 0), 1), ((1, 1), 1)], [((1, 0), 1), ((1, 1), 1)], [((0, 0), 1)], [((1, 1), 1)],
       [((0, 0), 1), ((0, 1), 1)], [((1, 0), 1), ((0, 0), -1)], [((0, 1), 1), ((1, 1), -1)]]
_SB = [[((0, 0), 1), ((1, 1), 1)], [((0, 0), 1)], [((0, 1), 1), ((1, 1), -1)], [((1, 0), 1), ((0, 0), -1)],
       [((1, 1), 1)], [((0, 0), 1), ((0, 1), 1)], [((1, 0), 1), ((1, 1), 1)]]
_SC = {(0, 0): [(0, 1), (3, 1), (4, -1), (6, 1)], (0, 1): [(2, 1), (4, 1)],
       (1, 0): [(1, 1), (3, 1)], (1, 1): [(0, 1), (1, -1), (2, 1), (5, 1)]}
_ORDER = [2, 4, 0, 3, 6, 1, 5]


def _lhs_terms(p):
    t = [((o[0] * 2 + i[0], o[1] * 2 + i[1]), so * si)
         for (o, so) in _SA[p // 7] for (i, si) in _SA[p % 7]]
    return [t[0], t[3], t[1], t[2]] if len(t) == 4 else t


def _signed_sum(get, terms):
    assert terms[0][1] > 0
    acc = get(terms[0][0])
    for idx, sgn in terms[1:]:
        acc = acc + get(idx) if sgn > 0 else acc - get(idx)
    return acc


@jax.jit
def pallas_concat_heads__gqa_block_cached__gqa_block_cached__near_ridge_kernel(
    A_x: jax.Array,
    A_k_cache: jax.Array,
    A_v_cache: jax.Array,
    A_wq: jax.Array,
    A_wo: jax.Array,
    B_x: jax.Array,
    B_k_cache: jax.Array,
    B_v_cache: jax.Array,
    B_wq: jax.Array,
    B_wo: jax.Array,
):
    B, S, D = A_x.shape
    _, H, SK, DH = A_k_cache.shape
    assert (B, S, D, H, SK, DH) == (32, 48, 512, 32, 48, 128) and A_wq.shape == (D, H * DH)
    M = B * S
    R = 2 * S
    GQ, SW = 8, 4
    GA, HQ = 16, 8
    NQ, NS, NA, NHQ, NSL = H // GQ, GQ // SW, H // GA, GA // HQ, H // HQ
    assert GQ == HQ and NA == 2
    NB, NP = 4, 49
    NC = M // (NB * R)
    KB, NW, HPB = HQ * DH // NB, D // NB, HQ // NB
    TT = 16
    NTU, TPI = 2 * NSL, 3
    FR = 192
    QR = M - FR
    QC = 4
    STAGES = ((192, 2), (384, 2), (528, 3), (768, 5), (QR, GQ))
    LAG, GO, FSP, CSP, NG = 4, 3, 3, 2, 21
    cexp = (DH ** -0.5) * math.log2(math.e)
    porder = [o * 7 + i for o in _ORDER for i in _ORDER]
    SEM_Q, SEM_A = 0, 2 * NQ
    SEM_COLD = SEM_A + 2 * NA
    NSEM = SEM_COLD + len(STAGES) - 1

    def kernel(ax, ak, av, awq, awo, bx, bk, bv, bwq, bwo, out_hbm,
               x_s, k_s, v_s, wq_s, wo_s, q_s, t_s, d_s, m_s, c_s, p_s, out_s, sems):
        src = ((ax, ak, av, awq, awo), (bx, bk, bv, bwq, bwo))
        st = lambda i: i if isinstance(i, int) else 0

        def x_dma(br, lo, n, sem):
            return pltpu.make_async_copy(src[br][0].at[pl.ds(lo, n)], x_s.at[br, pl.ds(lo, n)],
                                         sems.at[sem])

        def wq_dmas(br, j, sem, h0=0, h1=GQ):
            out = []
            while h0 < h1:
                e = min(h1, (h0 // SW + 1) * SW)
                out.append(pltpu.make_async_copy(
                    src[st(br)][3].at[:, pl.ds((st(j) * GQ + h0) * DH, (e - h0) * DH)],
                    wq_s.at[br, j, h0 // SW, :, pl.ds((h0 % SW) * DH, (e - h0) * DH)],
                    sems.at[sem]))
                h0 = e
            return out

        def wo_dmas(br, sl, sem):
            rows = pl.ds(sl * HQ * DH, HQ * DH)
            if sl // NHQ == 0:
                return [pltpu.make_async_copy(src[st(br)][4].at[rows, :], wo_s.at[br, sl],
                                              sems.at[sem])]
            return [pltpu.make_async_copy(src[st(br)][4].at[rows, pl.ds((NB - 1 - nb) * NW, NW)],
                                          wo_s.at[br, sl, :, pl.ds(nb * NW, NW)], sems.at[sem])
                    for nb in range(NB)]

        def kv_dmas(br, j):
            t = br * NA + j
            hs = pl.ds(st(j) * GA, GA)
            return [pltpu.make_async_copy(src[st(br)][1].at[:, hs], k_s.at[t], sems.at[SEM_A + t]),
                    pltpu.make_async_copy(src[st(br)][2].at[:, hs], v_s.at[t], sems.at[SEM_A + t])]

        def out_dma(br, blk, c0=0, nc=D):
            rows = pl.ds(blk * R, R)
            return pltpu.make_async_copy(out_s.at[br, rows, pl.ds(c0, nc)],
                                         out_hbm.at[rows, pl.ds(br * D + c0, nc)], sems.at[SEM_Q + br])

        cold = []
        pr, ph = 0, 0
        for si, (r, h) in enumerate(STAGES):
            sem = SEM_Q if si == 0 else SEM_COLD + si - 1
            r = M if si == len(STAGES) - 1 else r
            cold.append(wq_dmas(0, 0, sem, ph, h) + [x_dma(0, pr, r - pr, sem)])
            pr, ph = r, h
        for grp in cold:
            for d in grp:
                d.start()
        for br in range(2):
            if br == 1:
                x_dma(1, 0, M, SEM_Q + NQ).start(priority=1)
            for j in range(NQ):
                if br + j == 0:
                    dmas = wo_dmas(0, 0, SEM_Q + 1)
                else:
                    dmas = wq_dmas(br, j, SEM_Q + br * NQ + j) + wo_dmas(br, j, SEM_Q + br * NQ + j)
                for d in dmas:
                    d.start(priority=1)
            for j in range(NA):
                for d in kv_dmas(br, j):
                    d.start(priority=1)

        mask = (lax.broadcasted_iota(jnp.int32, (R, DH), 0) // S
                == lax.broadcasted_iota(jnp.int32, (R, DH), 1) // S)

        def q_proj(br, j, r0, r1, h0, h1):
            while h0 < h1:
                e = min(h1, (h0 // SW + 1) * SW)
                w = wq_s[br, j, h0 // SW, :, (h0 % SW) * DH:(h0 % SW + e - h0) * DH]
                q = jnp.dot(x_s[br, r0:r1, :], w, preferred_element_type=F32)
                for h in range(h0, e):
                    q_s[j, h, r0:r1, :] = q[:, (h - h0) * DH:(h - h0 + 1) * DH].astype(BF)
                h0 = e
            return q

        def t_tile(br, u, r0, gates, always, dacc):
            sl, half = u
            lo = pl.multiple_of(half * DH + r0, TT)
            w = {}
            for kb in range(NB):
                rows = pl.ds(kb * KB + lo, TT)
                for nb in range(NB):
                    w[(kb, nb)] = wo_s[br, sl, rows, nb * NW:(nb + 1) * NW].astype(F32)
            diag = (lax.broadcasted_iota(jnp.int32, (TT, DH), 1)
                    == lax.broadcasted_iota(jnp.int32, (TT, DH), 0) + r0)
            for kb in range(NB):
                a = [jnp.abs(w[(kb, nb)]) for nb in range(NB)]
                d = jnp.sum((a[0] + a[1]) + (a[2] + a[3]), axis=-1, keepdims=True)
                d = jnp.clip(d, 2.0 ** -100, 2.0 ** 100)
                dinv = pl.reciprocal(d, approx=True)
                dinv = dinv * (2.0 - d * dinv)
                for nb in range(NB):
                    w[(kb, nb)] = w[(kb, nb)] * dinv
                part = jnp.where(diag, d, 0.0)
                dacc[kb] = part if r0 == 0 else dacc[kb] + part
                if r0 + TT == DH:
                    drow = jnp.sum(jnp.where(always, dacc[kb], gates[-1]), axis=0, keepdims=True)
                    d_s[sl, kb, half] = jnp.broadcast_to(drow, (8, DH))
            for o in range(7):
                ob = {ii: _signed_sum(lambda oi: w[(oi[0] * 2 + ii[0], oi[1] * 2 + ii[1])], _SB[o])
                      for ii in ((0, 0), (0, 1), (1, 0), (1, 1))}
                for i in range(7):
                    p = o * 7 + i
                    tv = jnp.where(always, _signed_sum(ob.get, _SB[i]), gates[p * len(gates) // NP])
                    t_s[sl, p, pl.ds(lo, TT), :] = tv.astype(BF)

        pr, ph = 0, 0
        for si, (r, h) in enumerate(STAGES):
            for d in cold[si]:
                d.wait()
            if ph > 0:
                q_proj(0, 0, pr, r, 0, ph)
            if h > ph:
                q_proj(0, 0, 0, r, ph, h)
            pr, ph = r, h
        for d in wo_dmas(0, 0, SEM_Q + 1):
            d.wait()

        def q_body(j, br):
            sem = SEM_Q + br * NQ + j
            for d in wq_dmas(br, j, sem):
                d.wait()
            pltpu.make_async_copy(wo_s.at[br, j], wo_s.at[br, j], sems.at[sem]).wait()
            rc = QR // QC
            tiles = [(k, r0) for k in range(TPI) for r0 in range(0, DH, TT)]
            per = len(tiles) // (NS * QC)
            slots = [(nt, r_) for nt in range(SW) for r_ in range(0, rc - TT + 1, TT)]
            always = j >= 0
            us = [jnp.where(br == 0, jnp.minimum((j - 1) * TPI + k, NTU - 1), 2 * j + min(k, 1))
                  for k in range(TPI)]
            us = [(u >> 1, u & 1) for u in us]
            dacc = {}
            for qi in range(NS * QC):
                h0, ri = (qi // QC) * SW, qi % QC
                q = q_proj(br, j, ri * rc, (ri + 1) * rc, h0, h0 + SW)
                for ti, (k, r0) in enumerate(tiles[qi * per:(qi + 1) * per]):
                    gates = []
                    for gi in range(NG):
                        nt, r_ = slots[(ti * NG + gi) * len(slots) // (per * NG)]
                        gates.append(q[r_:r_ + TT, nt * DH:(nt + 1) * DH])
                    t_tile(br, us[k], r0, gates, always, dacc)
            return br

        def ao_body(j, br):
            t = br * NA + j
            for d in kv_dmas(br, j):
                d.wait()
            always, step0 = j >= 0, j == 0
            final = [t == b_ * NA + NA - 1 for b_ in range(2)]
            sub = [j * NHQ + i for i in range(NHQ)]
            zpad = jnp.zeros((DH - R, DH), BF)
            chunks = [(ci, hq) for ci in range(NC) for hq in range(NHQ)]
            units = [(ci * NB + p, hq * HQ + h)
                     for (ci, hq) in chunks for p in range(NB) for h in range(HQ)]
            upc = NB * HQ
            soft, outs, hist, lastm = {}, {}, [], {}
            pending, cqueue, cdone, ctick = [], [], set(), [0]

            def qk(u):
                p, h = units[u]
                kk = jnp.concatenate([k_s[t, 2 * p:2 * p + 2, h].reshape(R, DH), zpad], axis=0)
                s = lax.dot_general(q_s[sub[h // GQ], h % GQ, p * R:(p + 1) * R, :], kk, _NT,
                                    preferred_element_type=F32)
                s = jnp.where(mask, s, -jnp.inf)
                e = jnp.exp2((s - jnp.max(s, axis=-1, keepdims=True)) * cexp)
                soft[u] = (e, pl.reciprocal(jnp.sum(e, axis=-1, keepdims=True), approx=True))

            def pv(u):
                p, h = units[u]
                vv = jnp.concatenate([v_s[t, 2 * p:2 * p + 2, h].reshape(R, DH), zpad], axis=0)
                e, rinv = soft.pop(u)
                if len(hist) >= GO:
                    e = jnp.where(always, e, hist[-GO])
                o = jnp.dot(e.astype(BF), vv, preferred_element_type=F32) * rinv
                o = o * d_s[sub[h // HQ], h % HQ // HPB, h % HPB, 0:1, :]
                hist.append(o)
                outs[(p, h)] = o

            def recombine(ci, rb, nb, terms, first, last, gate):
                blk = ci * NB + rb
                rows = pl.ds(blk * R, R)
                if first:
                    cv = jnp.where(step0, 0.0, c_s[0, NB - 1 - nb, rows, :])
                else:
                    cv = p_s[nb, pl.ds(rb * R, R), :]
                if gate is not None:
                    cv = jnp.where(always, cv, gate)
                for p, sgn in terms:
                    mv = lastm[p] if p in lastm else m_s[p, pl.ds((ci % 2) * R, R), :]
                    cv = cv + mv if sgn > 0 else cv - mv
                if not last:
                    p_s[nb, pl.ds(rb * R, R), :] = cv
                    return
                c_s[j, nb, rows, :] = cv
                out_s[br, rows, (NB - 1 - nb) * NW:(NB - nb) * NW] = cv.astype(BF)
                cdone.add((ci, rb, nb))
                fine = blk == M // R - 1
                if fine or all((ci, rb, n_) in cdone for n_ in range(NB)):
                    for b_ in range(2):
                        @pl.when(final[b_])
                        def _():
                            if fine:
                                out_dma(b_, blk, (NB - 1 - nb) * NW, NW).start()
                            else:
                                out_dma(b_, blk).start()

            def product(u, p):
                ci, hq = chunks[u]
                last_chunk = u == len(chunks) - 1
                blk = lambda idx: jnp.concatenate(
                    [outs[(ci * NB + idx[0], hq * HQ + idx[1] * HPB + h)] for h in range(HPB)], axis=1)
                a = _signed_sum(blk, _lhs_terms(p)).astype(BF)
                mv = jnp.dot(a, t_s[sub[hq], p], preferred_element_type=F32)
                ctick[0] += 1
                if cqueue and (ctick[0] >= CSP or last_chunk):
                    ctick[0] = 0
                    recombine(*cqueue.pop(0), mv)
                assert all(task[0] >= ci - 1 for task in cqueue)
                rs = pl.ds((ci % 2) * R, R)
                if hq > 0:
                    mv = mv + m_s[p, rs, :]
                if last_chunk and p in porder[-2:]:
                    assert all(task[0] == ci for task in cqueue)
                    lastm[p] = mv
                else:
                    m_s[p, rs, :] = mv
                if hq < NHQ - 1:
                    return
                o_, i_ = divmod(p, 7)
                for oblk, oterms in _SC.items():
                    oseq = sorted(oterms, key=lambda x: _ORDER.index(x[0]))
                    for pos, (ko, so) in enumerate(oseq):
                        if ko != o_:
                            continue
                        for iblk, iterms in _SC.items():
                            iseq = sorted(iterms, key=lambda x: _ORDER.index(x[0]))
                            if iseq[-1][0] == i_:
                                cqueue.append((ci, oblk[0] * 2 + iblk[0], oblk[1] * 2 + iblk[1],
                                               [(o_ * 7 + ki, so * si) for ki, si in iseq],
                                               pos == 0, pos == len(oseq) - 1))

            fill = list(range(GA))
            tick = [0]

            def filler():
                if fill and tick[0] % FSP == 0:
                    h = fill.pop(0)
                    q_proj(br, sub[h // GQ], QR, M, h % GQ, h % GQ + 1)
                tick[0] += 1

            for u in range(LAG):
                filler()
                qk(u)
            credit = 0.0
            for u in range(len(units)):
                filler()
                pv(u)
                if u + LAG < len(units):
                    assert not fill or (units[u + LAG][0] + 1) * R <= QR
                    qk(u + LAG)
                if (u + 1) % upc == 0:
                    pending += [(u // upc, p) for p in porder]
                credit += NP / upc
                n = int(credit + 1e-9)
                credit -= n
                for _ in range(min(n, len(pending))):
                    product(*pending.pop(0))
            while pending:
                product(*pending.pop(0))
            while cqueue:
                recombine(*cqueue.pop(0), None)
            return br

        def branch(br, carry):
            @pl.when(br == 1)
            def _():
                x_dma(1, 0, M, SEM_Q + NQ).wait()
            lax.fori_loop(1 - br, NQ, q_body, br)
            lax.fori_loop(0, NA, ao_body, br)
            return carry

        lax.fori_loop(0, 2, branch, 0)
        for b_ in range(2):
            for blk in range(M // R - 1):
                out_dma(b_, blk).wait()
            for nb in range(NB):
                out_dma(b_, M // R - 1, nb * NW, NW).wait()

    anyspec = pl.BlockSpec(memory_space=pl.ANY)
    out = pl.pallas_call(
        kernel,
        in_specs=[anyspec] * 10,
        out_specs=anyspec,
        out_shape=jax.ShapeDtypeStruct((M, 2 * D), BF),
        scratch_shapes=[
            pltpu.VMEM((2, M, D), BF),
            pltpu.VMEM((2 * NA, B, GA, S, DH), BF),
            pltpu.VMEM((2 * NA, B, GA, S, DH), BF),
            pltpu.VMEM((2, NQ, NS, D, SW * DH), BF),
            pltpu.VMEM((2, NSL, HQ * DH, D), BF),
            pltpu.VMEM((NQ, GQ, M, DH), BF),
            pltpu.VMEM((NSL, NP, KB, NW), BF),
            pltpu.VMEM((NSL, NB, HPB, 8, DH), F32),
            pltpu.VMEM((NP, 2 * R, NW), F32),
            pltpu.VMEM((NA, NB, M, NW), F32),
            pltpu.VMEM((NB, NB * R, NW), F32),
            pltpu.VMEM((2, M, D), BF),
            pltpu.SemaphoreType.DMA((NSEM,)),
        ],
        compiler_params=pltpu.CompilerParams(vmem_limit_bytes=120 * 1024 * 1024),
    )(A_x.reshape(M, D), A_k_cache, A_v_cache, A_wq, A_wo,
      B_x.reshape(M, D), B_k_cache, B_v_cache, B_wq, B_wo)
    return out.reshape(B, S, 2 * D)
```

```python
import math

import jax
import jax.numpy as jnp
from jax import lax
import jax.experimental.pallas as pl
import jax.experimental.pallas.tpu as pltpu

F32 = jnp.float32
BF = jnp.bfloat16
_NT = (((1,), (1,)), ((), ()))

_SA = [[((0, 0), 1), ((1, 1), -1)], [((1, 0), 1), ((1, 1), -1)], [((0, 0), 1)], [((1, 1), 1)],
       [((0, 0), 1), ((0, 1), -1)], [((1, 0), 1), ((0, 0), -1)], [((1, 1), 1), ((0, 1), -1)]]
_SB = [[((0, 0), 1), ((1, 1), 1)], [((0, 0), 1)], [((0, 1), 1), ((1, 1), 1)], [((1, 0), 1), ((0, 0), 1)],
       [((1, 1), 1)], [((0, 0), 1), ((0, 1), -1)], [((1, 1), 1), ((1, 0), -1)]]
_SC = {(0, 0): [(0, 1), (3, 1), (4, -1), (6, 1)], (0, 1): [(2, 1), (4, -1)],
       (1, 0): [(1, 1), (3, 1)], (1, 1): [(0, -1), (1, 1), (2, 1), (5, -1)]}
_SA_IN = [[((0, 0), 1), ((1, 1), 1)], [((1, 0), 1), ((1, 1), 1)], [((0, 0), 1)], [((1, 1), 1)],
          [((0, 0), 1), ((0, 1), 1)], [((1, 0), 1), ((0, 0), -1)], [((0, 1), 1), ((1, 1), -1)]]
_SB_IN = [[((0, 0), 1), ((1, 1), -1)], [((0, 0), 1)], [((0, 1), 1), ((1, 1), -1)], [((1, 0), 1), ((0, 0), -1)],
          [((1, 1), 1)], [((0, 0), 1), ((0, 1), -1)], [((1, 0), 1), ((1, 1), -1)]]
_SC_IN = {(0, 0): [(0, 1), (3, 1), (4, 1), (6, 1)], (0, 1): [(2, 1), (4, 1)],
          (1, 0): [(1, 1), (3, 1)], (1, 1): [(0, -1), (1, 1), (2, 1), (5, -1)]}
_ORDER = [2, 4, 0, 3, 6, 1, 5]


def _lhs_terms(p):
    t = [((o[0] * 2 + i[0], o[1] * 2 + i[1]), so * si)
         for (o, so) in _SA[p // 7] for (i, si) in _SA_IN[p % 7]]
    return [t[0], t[3], t[1], t[2]] if len(t) == 4 else t


def _signed_sum(get, terms):
    assert terms[0][1] > 0
    acc = get(terms[0][0])
    for idx, sgn in terms[1:]:
        acc = acc + get(idx) if sgn > 0 else acc - get(idx)
    return acc


@jax.jit
def pallas_concat_heads__gqa_block_cached__gqa_block_cached__near_ridge_kernel(
    A_x: jax.Array,
    A_k_cache: jax.Array,
    A_v_cache: jax.Array,
    A_wq: jax.Array,
    A_wo: jax.Array,
    B_x: jax.Array,
    B_k_cache: jax.Array,
    B_v_cache: jax.Array,
    B_wq: jax.Array,
    B_wo: jax.Array,
):
    B, S, D = A_x.shape
    _, H, SK, DH = A_k_cache.shape
    assert (B, S, D, H, SK, DH) == (32, 48, 512, 32, 48, 128) and A_wq.shape == (D, H * DH)
    M = B * S
    R = 2 * S
    GQ, SW = 8, 4
    GA, HQ = 16, 8
    NQ, NS, NA, NHQ, NSL = H // GQ, GQ // SW, H // GA, GA // HQ, H // HQ
    assert GQ == HQ and NA == 2
    NB, NP = 4, 49
    NC = M // (NB * R)
    KB, NW, HPB = HQ * DH // NB, D // NB, HQ // NB
    TT = 16
    NTU, TPI = 2 * NSL, 3
    FR = 160
    QR = M - FR
    QC = 2
    STAGES = ((192, 2), (384, 2), (528, 3), (768, 5), (QR, GQ))
    LAG, GO, FSP, CSP, NG = 4, 3, 3, 2, 21
    cexp = (DH ** -0.5) * math.log2(math.e)
    porder = [o * 7 + i for o in _ORDER for i in _ORDER]
    SEM_Q, SEM_A = 0, 2 * NQ
    SEM_COLD = SEM_A + 2 * NA
    NSEM = SEM_COLD + len(STAGES) - 1

    def kernel(ax, ak, av, awq, awo, bx, bk, bv, bwq, bwo, out_hbm,
               x_s, k_s, v_s, wq_s, wo_s, q_s, t_s, d_s, m_s, c_s, p_s, out_s, sems):
        src = ((ax, ak, av, awq, awo), (bx, bk, bv, bwq, bwo))
        st = lambda i: i if isinstance(i, int) else 0

        def x_dma(br, lo, n, sem):
            return pltpu.make_async_copy(src[br][0].at[pl.ds(lo, n)], x_s.at[br, pl.ds(lo, n)],
                                         sems.at[sem])

        def wq_dmas(br, j, sem, h0=0, h1=GQ):
            out = []
            while h0 < h1:
                e = min(h1, (h0 // SW + 1) * SW)
                out.append(pltpu.make_async_copy(
                    src[st(br)][3].at[:, pl.ds((st(j) * GQ + h0) * DH, (e - h0) * DH)],
                    wq_s.at[br, j, h0 // SW, :, pl.ds((h0 % SW) * DH, (e - h0) * DH)],
                    sems.at[sem]))
                h0 = e
            return out

        def wo_dmas(br, sl, sem):
            rows = pl.ds(sl * HQ * DH, HQ * DH)
            if sl // NHQ == 0:
                return [pltpu.make_async_copy(src[st(br)][4].at[rows, :], wo_s.at[br, sl],
                                              sems.at[sem])]
            return [pltpu.make_async_copy(src[st(br)][4].at[rows, pl.ds((NB - 1 - nb) * NW, NW)],
                                          wo_s.at[br, sl, :, pl.ds(nb * NW, NW)], sems.at[sem])
                    for nb in range(NB)]

        def kv_dmas(br, j):
            t = br * NA + j
            hs = pl.ds(st(j) * GA, GA)
            return [pltpu.make_async_copy(src[st(br)][1].at[:, hs], k_s.at[t], sems.at[SEM_A + t]),
                    pltpu.make_async_copy(src[st(br)][2].at[:, hs], v_s.at[t], sems.at[SEM_A + t])]

        def out_dma(br, blk, c0=0, nc=D):
            rows = pl.ds(blk * R, R)
            return pltpu.make_async_copy(out_s.at[br, rows, pl.ds(c0, nc)],
                                         out_hbm.at[rows, pl.ds(br * D + c0, nc)], sems.at[SEM_Q + br])

        cold = []
        pr, ph = 0, 0
        for si, (r, h) in enumerate(STAGES):
            sem = SEM_Q if si == 0 else SEM_COLD + si - 1
            r = M if si == len(STAGES) - 1 else r
            cold.append(wq_dmas(0, 0, sem, ph, h) + [x_dma(0, pr, r - pr, sem)])
            pr, ph = r, h
        for grp in cold:
            for d in grp:
                d.start()
        for br in range(2):
            if br == 1:
                x_dma(1, 0, M, SEM_Q + NQ).start(priority=1)
            for j in range(NQ):
                if br + j == 0:
                    dmas = wo_dmas(0, 0, SEM_Q + 1)
                else:
                    dmas = wq_dmas(br, j, SEM_Q + br * NQ + j) + wo_dmas(br, j, SEM_Q + br * NQ + j)
                for d in dmas:
                    d.start(priority=1)
            for j in range(NA):
                for d in kv_dmas(br, j):
                    d.start(priority=1)

        mask = (lax.broadcasted_iota(jnp.int32, (R, DH), 0) // S
                == lax.broadcasted_iota(jnp.int32, (R, DH), 1) // S)

        def q_proj(br, j, r0, r1, h0, h1):
            while h0 < h1:
                e = min(h1, (h0 // SW + 1) * SW)
                w = wq_s[br, j, h0 // SW, :, (h0 % SW) * DH:(h0 % SW + e - h0) * DH]
                q = jnp.dot(x_s[br, r0:r1, :], w, preferred_element_type=F32)
                for h in range(h0, e):
                    q_s[j, h, r0:r1, :] = q[:, (h - h0) * DH:(h - h0 + 1) * DH].astype(BF)
                h0 = e
            return q

        def t_tile(br, u, r0, gates, always, dacc):
            sl, half = u
            lo = pl.multiple_of(half * DH + r0, TT)
            w = {}
            for kb in range(NB):
                rows = pl.ds(kb * KB + lo, TT)
                for nb in range(NB):
                    w[(kb, nb)] = wo_s[br, sl, rows, nb * NW:(nb + 1) * NW].astype(F32)
            diag = (lax.broadcasted_iota(jnp.int32, (TT, DH), 1)
                    == lax.broadcasted_iota(jnp.int32, (TT, DH), 0) + r0)
            for kb in range(NB):
                a = [jnp.abs(w[(kb, nb)]) for nb in range(NB)]
                d = jnp.sum((a[0] + a[1]) + (a[2] + a[3]), axis=-1, keepdims=True)
                d = jnp.clip(d, 2.0 ** -100, 2.0 ** 100)
                dinv = pl.reciprocal(d, approx=True)
                dinv = dinv * (2.0 - d * dinv)
                for nb in range(NB):
                    w[(kb, nb)] = w[(kb, nb)] * dinv
                part = jnp.where(diag, d, 0.0)
                dacc[kb] = part if r0 == 0 else dacc[kb] + part
                if r0 + TT == DH:
                    drow = jnp.sum(jnp.where(always, dacc[kb], gates[-1]), axis=0, keepdims=True)
                    d_s[sl, kb, half] = jnp.broadcast_to(drow, (8, DH))
            for o in range(7):
                ob = {ii: _signed_sum(lambda oi: w[(oi[0] * 2 + ii[0], oi[1] * 2 + ii[1])], _SB[o])
                      for ii in ((0, 0), (0, 1), (1, 0), (1, 1))}
                for i in range(7):
                    p = o * 7 + i
                    tv = jnp.where(always, _signed_sum(ob.get, _SB_IN[i]), gates[p * len(gates) // NP])
                    t_s[sl, p, pl.ds(lo, TT), :] = tv.astype(BF)

        pr, ph = 0, 0
        for si, (r, h) in enumerate(STAGES):
            for d in cold[si]:
                d.wait()
            if ph > 0:
                q_proj(0, 0, pr, r, 0, ph)
            if h > ph:
                q_proj(0, 0, 0, r, ph, h)
            pr, ph = r, h
        for d in wo_dmas(0, 0, SEM_Q + 1):
            d.wait()

        def q_body(j, br):
            sem = SEM_Q + br * NQ + j
            for d in wq_dmas(br, j, sem):
                d.wait()
            pltpu.make_async_copy(wo_s.at[br, j], wo_s.at[br, j], sems.at[sem]).wait()
            rc = QR // QC
            tiles = [(k, r0) for k in range(TPI) for r0 in range(0, DH, TT)]
            per = len(tiles) // (NS * QC)
            slots = [(nt, r_) for nt in range(SW) for r_ in range(0, rc - TT + 1, TT)]
            always = j >= 0
            us = [jnp.where(br == 0, jnp.minimum((j - 1) * TPI + k, NTU - 1), 2 * j + min(k, 1))
                  for k in range(TPI)]
            us = [(u >> 1, u & 1) for u in us]
            dacc = {}
            for qi in range(NS * QC):
                h0, ri = (qi // QC) * SW, qi % QC
                q = q_proj(br, j, ri * rc, (ri + 1) * rc, h0, h0 + SW)
                for ti, (k, r0) in enumerate(tiles[qi * per:(qi + 1) * per]):
                    gates = []
                    for gi in range(NG):
                        nt, r_ = slots[(ti * NG + gi) * len(slots) // (per * NG)]
                        gates.append(q[r_:r_ + TT, nt * DH:(nt + 1) * DH])
                    t_tile(br, us[k], r0, gates, always, dacc)
            return br

        def ao_body(j, br):
            t = br * NA + j
            for d in kv_dmas(br, j):
                d.wait()
            always, step0 = j >= 0, j == 0
            final = [t == b_ * NA + NA - 1 for b_ in range(2)]
            sub = [j * NHQ + i for i in range(NHQ)]
            zpad = jnp.zeros((DH - R, DH), BF)
            chunks = [(ci, hq) for ci in range(NC) for hq in range(NHQ)]
            units = [(ci * NB + p, hq * HQ + h)
                     for (ci, hq) in chunks for p in range(NB) for h in range(HQ)]
            upc = NB * HQ
            soft, outs, hist, lastm = {}, {}, [], {}
            pending, cqueue, cdone, ctick = [], [], set(), [0]

            def qk(u):
                p, h = units[u]
                kk = jnp.concatenate([k_s[t, 2 * p:2 * p + 2, h].reshape(R, DH), zpad], axis=0)
                s = lax.dot_general(q_s[sub[h // GQ], h % GQ, p * R:(p + 1) * R, :], kk, _NT,
                                    preferred_element_type=F32)
                s = jnp.where(mask, s, -jnp.inf)
                e = jnp.exp2((s - jnp.max(s, axis=-1, keepdims=True)) * cexp)
                soft[u] = (e, pl.reciprocal(jnp.sum(e, axis=-1, keepdims=True), approx=True))

            def pv(u):
                p, h = units[u]
                vv = jnp.concatenate([v_s[t, 2 * p:2 * p + 2, h].reshape(R, DH), zpad], axis=0)
                e, rinv = soft.pop(u)
                if len(hist) >= GO:
                    e = jnp.where(always, e, hist[-GO])
                o = jnp.dot(e.astype(BF), vv, preferred_element_type=F32) * rinv
                o = o * d_s[sub[h // HQ], h % HQ // HPB, h % HPB, 0:1, :]
                hist.append(o)
                outs[(p, h)] = o

            def recombine(ci, rb, nb, terms, first, last, gate):
                blk = ci * NB + rb
                rows = pl.ds(blk * R, R)
                if first:
                    cv = jnp.where(step0, 0.0, c_s[0, NB - 1 - nb, rows, :])
                else:
                    cv = p_s[nb, pl.ds(rb * R, R), :]
                if gate is not None:
                    cv = jnp.where(always, cv, gate)
                for p, sgn in terms:
                    mv = lastm[p] if p in lastm else m_s[p, pl.ds((ci % 2) * R, R), :]
                    cv = cv + mv if sgn > 0 else cv - mv
                if not last:
                    p_s[nb, pl.ds(rb * R, R), :] = cv
                    return
                c_s[j, nb, rows, :] = cv
                out_s[br, rows, (NB - 1 - nb) * NW:(NB - nb) * NW] = cv.astype(BF)
                cdone.add((ci, rb, nb))
                fine = blk == M // R - 1
                if fine or all((ci, rb, n_) in cdone for n_ in range(NB)):
                    for b_ in range(2):
                        @pl.when(final[b_])
                        def _():
                            if fine:
                                out_dma(b_, blk, (NB - 1 - nb) * NW, NW).start()
                            else:
                                out_dma(b_, blk).start()

            def product(u, p):
                ci, hq = chunks[u]
                last_chunk = u == len(chunks) - 1
                blk = lambda idx: jnp.concatenate(
                    [outs[(ci * NB + idx[0], hq * HQ + idx[1] * HPB + h)] for h in range(HPB)], axis=1)
                a = _signed_sum(blk, _lhs_terms(p)).astype(BF)
                mv = jnp.dot(a, t_s[sub[hq], p], preferred_element_type=F32)
                ctick[0] += 1
                if cqueue and (ctick[0] >= CSP or last_chunk):
                    ctick[0] = 0
                    recombine(*cqueue.pop(0), mv)
                assert all(task[0] >= ci - 1 for task in cqueue)
                rs = pl.ds((ci % 2) * R, R)
                if hq > 0:
                    mv = mv + m_s[p, rs, :]
                if last_chunk and p in porder[-2:]:
                    assert all(task[0] == ci for task in cqueue)
                    lastm[p] = mv
                else:
                    m_s[p, rs, :] = mv
                if hq < NHQ - 1:
                    return
                o_, i_ = divmod(p, 7)
                for oblk, oterms in _SC.items():
                    oseq = sorted(oterms, key=lambda x: _ORDER.index(x[0]))
                    for pos, (ko, so) in enumerate(oseq):
                        if ko != o_:
                            continue
                        for iblk, iterms in _SC_IN.items():
                            iseq = sorted(iterms, key=lambda x: _ORDER.index(x[0]))
                            if iseq[-1][0] == i_:
                                cqueue.append((ci, oblk[0] * 2 + iblk[0], oblk[1] * 2 + iblk[1],
                                               [(o_ * 7 + ki, so * si) for ki, si in iseq],
                                               pos == 0, pos == len(oseq) - 1))

            fill = list(range(GA))
            tick = [0]

            def filler():
                if fill and tick[0] % FSP == 0:
                    h = fill.pop(0)
                    q_proj(br, sub[h // GQ], QR, M, h % GQ, h % GQ + 1)
                tick[0] += 1

            for u in range(LAG):
                filler()
                qk(u)
            credit = 0.0
            for u in range(len(units)):
                filler()
                pv(u)
                if u + LAG < len(units):
                    assert not fill or (units[u + LAG][0] + 1) * R <= QR
                    qk(u + LAG)
                if (u + 1) % upc == 0:
                    pending += [(u // upc, p) for p in porder]
                credit += NP / upc
                n = int(credit + 1e-9)
                credit -= n
                for _ in range(min(n, len(pending))):
                    product(*pending.pop(0))
            while pending:
                product(*pending.pop(0))
            while cqueue:
                recombine(*cqueue.pop(0), None)
            return br

        def branch(br, carry):
            @pl.when(br == 1)
            def _():
                x_dma(1, 0, M, SEM_Q + NQ).wait()
            lax.fori_loop(1 - br, NQ, q_body, br)
            lax.fori_loop(0, NA, ao_body, br)
            return carry

        lax.fori_loop(0, 2, branch, 0)
        for b_ in range(2):
            for blk in range(M // R - 1):
                out_dma(b_, blk).wait()
            for nb in range(NB):
                out_dma(b_, M // R - 1, nb * NW, NW).wait()

    anyspec = pl.BlockSpec(memory_space=pl.ANY)
    out = pl.pallas_call(
        kernel,
        in_specs=[anyspec] * 10,
        out_specs=anyspec,
        out_shape=jax.ShapeDtypeStruct((M, 2 * D), BF),
        scratch_shapes=[
            pltpu.VMEM((2, M, D), BF),
            pltpu.VMEM((2 * NA, B, GA, S, DH), BF),
            pltpu.VMEM((2 * NA, B, GA, S, DH), BF),
            pltpu.VMEM((2, NQ, NS, D, SW * DH), BF),
            pltpu.VMEM((2, NSL, HQ * DH, D), BF),
            pltpu.VMEM((NQ, GQ, M, DH), BF),
            pltpu.VMEM((NSL, NP, KB, NW), BF),
            pltpu.VMEM((NSL, NB, HPB, 8, DH), F32),
            pltpu.VMEM((NP, 2 * R, NW), F32),
            pltpu.VMEM((NA, NB, M, NW), F32),
            pltpu.VMEM((NB, NB * R, NW), F32),
            pltpu.VMEM((2, M, D), BF),
            pltpu.SemaphoreType.DMA((NSEM,)),
        ],
        compiler_params=pltpu.CompilerParams(vmem_limit_bytes=120 * 1024 * 1024),
    )(A_x.reshape(M, D), A_k_cache, A_v_cache, A_wq, A_wo,
      B_x.reshape(M, D), B_k_cache, B_v_cache, B_wq, B_wo)
    return out.reshape(B, S, 2 * D)
```

```python
import math

import jax
import jax.numpy as jnp
from jax import lax
import jax.experimental.pallas as pl
import jax.experimental.pallas.tpu as pltpu

F32 = jnp.float32
BF = jnp.bfloat16
_NT = (((1,), (1,)), ((), ()))

_SA = [[((0, 0), 1), ((1, 1), -1)], [((1, 0), 1), ((1, 1), -1)], [((0, 0), 1)], [((1, 1), 1)],
       [((0, 0), 1), ((0, 1), -1)], [((1, 0), 1), ((0, 0), -1)], [((1, 1), 1), ((0, 1), -1)]]
_SB = [[((0, 0), 1), ((1, 1), 1)], [((0, 0), 1)], [((0, 1), 1), ((1, 1), 1)], [((1, 0), 1), ((0, 0), 1)],
       [((1, 1), 1)], [((0, 0), 1), ((0, 1), -1)], [((1, 1), 1), ((1, 0), -1)]]
_SC = {(0, 0): [(0, 1), (3, 1), (4, -1), (6, 1)], (0, 1): [(2, 1), (4, -1)],
       (1, 0): [(1, 1), (3, 1)], (1, 1): [(0, -1), (1, 1), (2, 1), (5, -1)]}
_SA_IN = [[((0, 0), 1), ((1, 1), 1)], [((1, 0), 1), ((1, 1), 1)], [((0, 0), 1)], [((1, 1), 1)],
          [((0, 0), 1), ((0, 1), 1)], [((1, 0), 1), ((0, 0), -1)], [((0, 1), 1), ((1, 1), -1)]]
_SB_IN = [[((0, 0), 1), ((1, 1), -1)], [((0, 0), 1)], [((0, 1), 1), ((1, 1), -1)], [((1, 0), 1), ((0, 0), -1)],
          [((1, 1), 1)], [((0, 0), 1), ((0, 1), -1)], [((1, 0), 1), ((1, 1), -1)]]
_SC_IN = {(0, 0): [(0, 1), (3, 1), (4, 1), (6, 1)], (0, 1): [(2, 1), (4, 1)],
          (1, 0): [(1, 1), (3, 1)], (1, 1): [(0, -1), (1, 1), (2, 1), (5, -1)]}
_ORDER = [2, 4, 0, 3, 6, 1, 5]


def _lhs_terms(p):
    t = [((o[0] * 2 + i[0], o[1] * 2 + i[1]), so * si)
         for (o, so) in _SA[p // 7] for (i, si) in _SA_IN[p % 7]]
    return [t[0], t[3], t[1], t[2]] if len(t) == 4 else t


def _signed_sum(get, terms):
    assert terms[0][1] > 0
    acc = get(terms[0][0])
    for idx, sgn in terms[1:]:
        acc = acc + get(idx) if sgn > 0 else acc - get(idx)
    return acc


@jax.jit
def pallas_concat_heads__gqa_block_cached__gqa_block_cached__near_ridge_kernel(
    A_x: jax.Array,
    A_k_cache: jax.Array,
    A_v_cache: jax.Array,
    A_wq: jax.Array,
    A_wo: jax.Array,
    B_x: jax.Array,
    B_k_cache: jax.Array,
    B_v_cache: jax.Array,
    B_wq: jax.Array,
    B_wo: jax.Array,
):
    B, S, D = A_x.shape
    _, H, SK, DH = A_k_cache.shape
    assert (B, S, D, H, SK, DH) == (32, 48, 512, 32, 48, 128) and A_wq.shape == (D, H * DH)
    M = B * S
    R = 2 * S
    GQ, SW = 8, 4
    GA, HQ = 16, 8
    NQ, NS, NA, NHQ, NSL = H // GQ, GQ // SW, H // GA, GA // HQ, H // HQ
    assert GQ == HQ and NA == 2
    NB, NP = 4, 49
    NC = M // (NB * R)
    KB, NW, HPB = HQ * DH // NB, D // NB, HQ // NB
    TT = 16
    NTU, TPI = 2 * NSL, 3
    FR = 160
    QR = M - FR
    QC = 2
    STAGES = ((192, 2), (384, 2), (528, 3), (768, 5), (QR, GQ))
    LAG, GO, FSP, CSP, NG = 4, 3, 3, 2, 21
    cexp = (DH ** -0.5) * math.log2(math.e)
    porder = [o * 7 + i for o in _ORDER for i in _ORDER]
    SEM_Q, SEM_A = 0, 2 * NQ
    SEM_COLD = SEM_A + 2 * NA
    NSEM = SEM_COLD + len(STAGES) - 1

    def kernel(ax, ak, av, awq, awo, bx, bk, bv, bwq, bwo, out_hbm,
               x_s, k_s, v_s, wq_s, wo_s, q_s, t_s, d_s, m_s, c_s, p_s, out_s, sems):
        src = ((ax, ak, av, awq, awo), (bx, bk, bv, bwq, bwo))
        st = lambda i: i if isinstance(i, int) else 0

        def x_dma(br, lo, n, sem):
            return pltpu.make_async_copy(src[br][0].at[pl.ds(lo, n)], x_s.at[br, pl.ds(lo, n)],
                                         sems.at[sem])

        def wq_dmas(br, j, sem, h0=0, h1=GQ):
            out = []
            while h0 < h1:
                e = min(h1, (h0 // SW + 1) * SW)
                out.append(pltpu.make_async_copy(
                    src[st(br)][3].at[:, pl.ds((st(j) * GQ + h0) * DH, (e - h0) * DH)],
                    wq_s.at[br, j, h0 // SW, :, pl.ds((h0 % SW) * DH, (e - h0) * DH)],
                    sems.at[sem]))
                h0 = e
            return out

        def wo_dmas(br, sl, sem):
            rows = pl.ds(sl * HQ * DH, HQ * DH)
            if sl // NHQ == 0:
                return [pltpu.make_async_copy(src[st(br)][4].at[rows, :], wo_s.at[br, sl],
                                              sems.at[sem])]
            return [pltpu.make_async_copy(src[st(br)][4].at[rows, pl.ds((NB - 1 - nb) * NW, NW)],
                                          wo_s.at[br, sl, :, pl.ds(nb * NW, NW)], sems.at[sem])
                    for nb in range(NB)]

        def kv_dmas(br, j):
            t = br * NA + j
            hs = pl.ds(st(j) * GA, GA)
            return [pltpu.make_async_copy(src[st(br)][1].at[:, hs], k_s.at[t], sems.at[SEM_A + t]),
                    pltpu.make_async_copy(src[st(br)][2].at[:, hs], v_s.at[t], sems.at[SEM_A + t])]

        def out_dma(br, blk, nblk, nb):
            rows = pl.ds(blk * R, nblk * R)
            return pltpu.make_async_copy(out_s.at[br, nb, rows],
                                         out_hbm.at[rows, pl.ds(br * D + nb * NW, NW)], sems.at[SEM_Q + br])

        cold = []
        pr, ph = 0, 0
        for si, (r, h) in enumerate(STAGES):
            sem = SEM_Q if si == 0 else SEM_COLD + si - 1
            r = M if si == len(STAGES) - 1 else r
            cold.append(wq_dmas(0, 0, sem, ph, h) + [x_dma(0, pr, r - pr, sem)])
            pr, ph = r, h
        for grp in cold:
            for d in grp:
                d.start()
        for br in range(2):
            if br == 1:
                x_dma(1, 0, M, SEM_Q + NQ).start(priority=1)
            for j in range(NQ):
                if br + j == 0:
                    dmas = wo_dmas(0, 0, SEM_Q + 1)
                else:
                    dmas = wq_dmas(br, j, SEM_Q + br * NQ + j) + wo_dmas(br, j, SEM_Q + br * NQ + j)
                for d in dmas:
                    d.start(priority=1)
            for j in range(NA):
                for d in kv_dmas(br, j):
                    d.start(priority=1)

        mask = (lax.broadcasted_iota(jnp.int32, (R, DH), 0) // S
                == lax.broadcasted_iota(jnp.int32, (R, DH), 1) // S)

        def q_proj(br, j, r0, r1, h0, h1):
            while h0 < h1:
                e = min(h1, (h0 // SW + 1) * SW)
                w = wq_s[br, j, h0 // SW, :, (h0 % SW) * DH:(h0 % SW + e - h0) * DH]
                q = jnp.dot(x_s[br, r0:r1, :], w, preferred_element_type=F32)
                for h in range(h0, e):
                    q_s[j, h, r0:r1, :] = q[:, (h - h0) * DH:(h - h0 + 1) * DH].astype(BF)
                h0 = e
            return q

        def t_tile(br, u, r0, gates, always, dacc):
            sl, half = u
            lo = pl.multiple_of(half * DH + r0, TT)
            w = {}
            for kb in range(NB):
                rows = pl.ds(kb * KB + lo, TT)
                for nb in range(NB):
                    w[(kb, nb)] = wo_s[br, sl, rows, nb * NW:(nb + 1) * NW].astype(F32)
            diag = (lax.broadcasted_iota(jnp.int32, (TT, DH), 1)
                    == lax.broadcasted_iota(jnp.int32, (TT, DH), 0) + r0)
            for kb in range(NB):
                a = [jnp.abs(w[(kb, nb)]) for nb in range(NB)]
                d = jnp.sum((a[0] + a[1]) + (a[2] + a[3]), axis=-1, keepdims=True)
                d = jnp.clip(d, 2.0 ** -100, 2.0 ** 100)
                dinv = pl.reciprocal(d, approx=True)
                dinv = dinv * (2.0 - d * dinv)
                for nb in range(NB):
                    w[(kb, nb)] = w[(kb, nb)] * dinv
                part = jnp.where(diag, d, 0.0)
                dacc[kb] = part if r0 == 0 else dacc[kb] + part
                if r0 + TT == DH:
                    drow = jnp.sum(jnp.where(always, dacc[kb], gates[-1]), axis=0, keepdims=True)
                    d_s[sl, kb, half] = jnp.broadcast_to(drow, (8, DH))
            for o in range(7):
                ob = {ii: _signed_sum(lambda oi: w[(oi[0] * 2 + ii[0], oi[1] * 2 + ii[1])], _SB[o])
                      for ii in ((0, 0), (0, 1), (1, 0), (1, 1))}
                for i in range(7):
                    p = o * 7 + i
                    tv = jnp.where(always, _signed_sum(ob.get, _SB_IN[i]), gates[p * len(gates) // NP])
                    t_s[sl, p, pl.ds(lo, TT), :] = tv.astype(BF)

        pr, ph = 0, 0
        for si, (r, h) in enumerate(STAGES):
            for d in cold[si]:
                d.wait()
            if ph > 0:
                q_proj(0, 0, pr, r, 0, ph)
            if h > ph:
                q_proj(0, 0, 0, r, ph, h)
            pr, ph = r, h
        for d in wo_dmas(0, 0, SEM_Q + 1):
            d.wait()

        def q_body(j, br):
            sem = SEM_Q + br * NQ + j
            for d in wq_dmas(br, j, sem):
                d.wait()
            pltpu.make_async_copy(wo_s.at[br, j], wo_s.at[br, j], sems.at[sem]).wait()
            rc = QR // QC
            tiles = [(k, r0) for k in range(TPI) for r0 in range(0, DH, TT)]
            per = len(tiles) // (NS * QC)
            slots = [(nt, r_) for nt in range(SW) for r_ in range(0, rc - TT + 1, TT)]
            always = j >= 0
            us = [jnp.where(br == 0, jnp.minimum((j - 1) * TPI + k, NTU - 1), 2 * j + min(k, 1))
                  for k in range(TPI)]
            us = [(u >> 1, u & 1) for u in us]
            dacc = {}
            for qi in range(NS * QC):
                h0, ri = (qi // QC) * SW, qi % QC
                q = q_proj(br, j, ri * rc, (ri + 1) * rc, h0, h0 + SW)
                for ti, (k, r0) in enumerate(tiles[qi * per:(qi + 1) * per]):
                    gates = []
                    for gi in range(NG):
                        nt, r_ = slots[(ti * NG + gi) * len(slots) // (per * NG)]
                        gates.append(q[r_:r_ + TT, nt * DH:(nt + 1) * DH])
                    t_tile(br, us[k], r0, gates, always, dacc)
            return br

        def ao_body(j, br):
            t = br * NA + j
            for d in kv_dmas(br, j):
                d.wait()
            always, step0 = j >= 0, j == 0
            final = [t == b_ * NA + NA - 1 for b_ in range(2)]
            sub = [j * NHQ + i for i in range(NHQ)]
            zpad = jnp.zeros((DH - R, DH), BF)
            chunks = [(ci, hq) for ci in range(NC) for hq in range(NHQ)]
            units = [(ci * NB + p, hq * HQ + h)
                     for (ci, hq) in chunks for p in range(NB) for h in range(HQ)]
            upc = NB * HQ
            soft, outs, hist, lastm = {}, {}, [], {}
            pending, cqueue, cdone, ctick = [], [], set(), [0]

            def qk(u):
                p, h = units[u]
                kk = jnp.concatenate([k_s[t, 2 * p:2 * p + 2, h].reshape(R, DH), zpad], axis=0)
                s = lax.dot_general(q_s[sub[h // GQ], h % GQ, p * R:(p + 1) * R, :], kk, _NT,
                                    preferred_element_type=F32)
                s = jnp.where(mask, s, -jnp.inf)
                e = jnp.exp2((s - jnp.max(s, axis=-1, keepdims=True)) * cexp)
                soft[u] = (e, pl.reciprocal(jnp.sum(e, axis=-1, keepdims=True), approx=True))

            def pv(u):
                p, h = units[u]
                vv = jnp.concatenate([v_s[t, 2 * p:2 * p + 2, h].reshape(R, DH), zpad], axis=0)
                e, rinv = soft.pop(u)
                if len(hist) >= GO:
                    e = jnp.where(always, e, hist[-GO])
                o = jnp.dot(e.astype(BF), vv, preferred_element_type=F32) * rinv
                o = o * d_s[sub[h // HQ], h % HQ // HPB, h % HPB, 0:1, :]
                hist.append(o)
                outs[(p, h)] = o

            def recombine(ci, rb, nb, terms, first, last, gate):
                rows = pl.ds((ci * NB + rb) * R, R)
                if first:
                    cv = jnp.where(step0, 0.0, c_s[0, NB - 1 - nb, rows, :])
                else:
                    cv = p_s[nb, pl.ds(rb * R, R), :]
                if gate is not None:
                    cv = jnp.where(always, cv, gate)
                for p, sgn in terms:
                    mv = lastm[p] if p in lastm else m_s[p, pl.ds((ci % 2) * R, R), :]
                    cv = cv + mv if sgn > 0 else cv - mv
                if not last:
                    p_s[nb, pl.ds(rb * R, R), :] = cv
                    return
                c_s[j, nb, rows, :] = cv
                out_s[br, NB - 1 - nb, rows, :] = cv.astype(BF)
                cdone.add((ci, rb, nb))
                g = 1 if ci == NC - 1 else NB
                r0 = rb // g * g
                if all((ci, r_, nb) in cdone for r_ in range(r0, r0 + g)):
                    for b_ in range(2):
                        @pl.when(final[b_])
                        def _():
                            out_dma(b_, ci * NB + r0, g, NB - 1 - nb).start()

            def product(u, p):
                ci, hq = chunks[u]
                last_chunk = u == len(chunks) - 1
                blk = lambda idx: jnp.concatenate(
                    [outs[(ci * NB + idx[0], hq * HQ + idx[1] * HPB + h)] for h in range(HPB)], axis=1)
                a = _signed_sum(blk, _lhs_terms(p)).astype(BF)
                mv = jnp.dot(a, t_s[sub[hq], p], preferred_element_type=F32)
                ctick[0] += 1
                if cqueue and (ctick[0] >= CSP or last_chunk):
                    ctick[0] = 0
                    recombine(*cqueue.pop(0), mv)
                assert all(task[0] >= ci - 1 for task in cqueue)
                rs = pl.ds((ci % 2) * R, R)
                if hq > 0:
                    mv = mv + m_s[p, rs, :]
                if last_chunk and p in porder[-2:]:
                    assert all(task[0] == ci for task in cqueue)
                    lastm[p] = mv
                else:
                    m_s[p, rs, :] = mv
                if hq < NHQ - 1:
                    return
                o_, i_ = divmod(p, 7)
                for oblk, oterms in _SC.items():
                    oseq = sorted(oterms, key=lambda x: _ORDER.index(x[0]))
                    for pos, (ko, so) in enumerate(oseq):
                        if ko != o_:
                            continue
                        for iblk, iterms in _SC_IN.items():
                            iseq = sorted(iterms, key=lambda x: _ORDER.index(x[0]))
                            if iseq[-1][0] == i_:
                                cqueue.append((ci, oblk[0] * 2 + iblk[0], oblk[1] * 2 + iblk[1],
                                               [(o_ * 7 + ki, so * si) for ki, si in iseq],
                                               pos == 0, pos == len(oseq) - 1))

            fill = list(range(GA))
            tick = [0]

            def filler():
                if fill and tick[0] % FSP == 0:
                    h = fill.pop(0)
                    q_proj(br, sub[h // GQ], QR, M, h % GQ, h % GQ + 1)
                tick[0] += 1

            for u in range(LAG):
                filler()
                qk(u)
            credit = 0.0
            for u in range(len(units)):
                filler()
                pv(u)
                if u + LAG < len(units):
                    assert not fill or (units[u + LAG][0] + 1) * R <= QR
                    qk(u + LAG)
                if (u + 1) % upc == 0:
                    pending += [(u // upc, p) for p in porder]
                credit += NP / upc
                n = int(credit + 1e-9)
                credit -= n
                for _ in range(min(n, len(pending))):
                    product(*pending.pop(0))
            while pending:
                product(*pending.pop(0))
            while cqueue:
                recombine(*cqueue.pop(0), None)
            return br

        def branch(br, carry):
            @pl.when(br == 1)
            def _():
                x_dma(1, 0, M, SEM_Q + NQ).wait()
            lax.fori_loop(1 - br, NQ, q_body, br)
            lax.fori_loop(0, NA, ao_body, br)
            return carry

        lax.fori_loop(0, 2, branch, 0)
        for b_ in range(2):
            for nb in range(NB):
                for ci in range(NC - 1):
                    out_dma(b_, ci * NB, NB, nb).wait()
                for rb in range(NB):
                    out_dma(b_, (NC - 1) * NB + rb, 1, nb).wait()

    anyspec = pl.BlockSpec(memory_space=pl.ANY)
    out = pl.pallas_call(
        kernel,
        in_specs=[anyspec] * 10,
        out_specs=anyspec,
        out_shape=jax.ShapeDtypeStruct((M, 2 * D), BF),
        scratch_shapes=[
            pltpu.VMEM((2, M, D), BF),
            pltpu.VMEM((2 * NA, B, GA, S, DH), BF),
            pltpu.VMEM((2 * NA, B, GA, S, DH), BF),
            pltpu.VMEM((2, NQ, NS, D, SW * DH), BF),
            pltpu.VMEM((2, NSL, HQ * DH, D), BF),
            pltpu.VMEM((NQ, GQ, M, DH), BF),
            pltpu.VMEM((NSL, NP, KB, NW), BF),
            pltpu.VMEM((NSL, NB, HPB, 8, DH), F32),
            pltpu.VMEM((NP, 2 * R, NW), F32),
            pltpu.VMEM((NA, NB, M, NW), F32),
            pltpu.VMEM((NB, NB * R, NW), F32),
            pltpu.VMEM((2, NB, M, NW), BF),
            pltpu.SemaphoreType.DMA((NSEM,)),
        ],
        compiler_params=pltpu.CompilerParams(vmem_limit_bytes=120 * 1024 * 1024),
    )(A_x.reshape(M, D), A_k_cache, A_v_cache, A_wq, A_wo,
      B_x.reshape(M, D), B_k_cache, B_v_cache, B_wq, B_wo)
    return out.reshape(B, S, 2 * D)
```

```python
import math

import jax
import jax.numpy as jnp
from jax import lax
import jax.experimental.pallas as pl
import jax.experimental.pallas.tpu as pltpu

F32 = jnp.float32
BF = jnp.bfloat16
_NT = (((1,), (1,)), ((), ()))

_SA = [[((0, 0), 1), ((1, 1), -1)], [((1, 0), 1), ((1, 1), -1)], [((0, 0), 1)], [((1, 1), 1)],
       [((0, 0), 1), ((0, 1), -1)], [((1, 0), 1), ((0, 0), -1)], [((1, 1), 1), ((0, 1), -1)]]
_SB = [[((0, 0), 1), ((1, 1), 1)], [((0, 0), 1)], [((0, 1), 1), ((1, 1), 1)], [((1, 0), 1), ((0, 0), 1)],
       [((1, 1), 1)], [((0, 0), 1), ((0, 1), -1)], [((1, 1), 1), ((1, 0), -1)]]
_SC = {(0, 0): [(0, 1), (3, 1), (4, -1), (6, 1)], (0, 1): [(2, 1), (4, -1)],
       (1, 0): [(1, 1), (3, 1)], (1, 1): [(0, -1), (1, 1), (2, 1), (5, -1)]}
_SA_IN = [[((0, 0), 1), ((1, 1), 1)], [((1, 0), 1), ((1, 1), 1)], [((0, 0), 1)], [((1, 1), 1)],
          [((0, 0), 1), ((0, 1), 1)], [((1, 0), 1), ((0, 0), -1)], [((0, 1), 1), ((1, 1), -1)]]
_SB_IN = [[((0, 0), 1), ((1, 1), -1)], [((0, 0), 1)], [((0, 1), 1), ((1, 1), -1)], [((1, 0), 1), ((0, 0), -1)],
          [((1, 1), 1)], [((0, 0), 1), ((0, 1), -1)], [((1, 0), 1), ((1, 1), -1)]]
_SC_IN = {(0, 0): [(0, 1), (3, 1), (4, 1), (6, 1)], (0, 1): [(2, 1), (4, 1)],
          (1, 0): [(1, 1), (3, 1)], (1, 1): [(0, -1), (1, 1), (2, 1), (5, -1)]}
_ORDER = [2, 4, 0, 3, 6, 1, 5]


def _lhs_terms(p):
    t = [((o[0] * 2 + i[0], o[1] * 2 + i[1]), so * si)
         for (o, so) in _SA[p // 7] for (i, si) in _SA_IN[p % 7]]
    return [t[0], t[3], t[1], t[2]] if len(t) == 4 else t


def _signed_sum(get, terms):
    assert terms[0][1] > 0
    acc = get(terms[0][0])
    for idx, sgn in terms[1:]:
        acc = acc + get(idx) if sgn > 0 else acc - get(idx)
    return acc


@jax.jit
def pallas_concat_heads__gqa_block_cached__gqa_block_cached__near_ridge_kernel(
    A_x: jax.Array,
    A_k_cache: jax.Array,
    A_v_cache: jax.Array,
    A_wq: jax.Array,
    A_wo: jax.Array,
    B_x: jax.Array,
    B_k_cache: jax.Array,
    B_v_cache: jax.Array,
    B_wq: jax.Array,
    B_wo: jax.Array,
):
    B, S, D = A_x.shape
    _, H, SK, DH = A_k_cache.shape
    assert (B, S, D, H, SK, DH) == (32, 48, 512, 32, 48, 128) and A_wq.shape == (D, H * DH)
    M = B * S
    R = 2 * S
    GQ, SW = 8, 4
    GA, HQ = 16, 8
    NQ, NS, NA, NHQ, NSL = H // GQ, GQ // SW, H // GA, GA // HQ, H // HQ
    assert GQ == HQ and NA == 2 and NS == NA
    NB, NP = 4, 49
    NC = M // (NB * R)
    KB, NW, HPB = HQ * DH // NB, D // NB, HQ // NB
    TT = 16
    NTU, TPI = 2 * NSL, 3
    FR = 160
    QR = M - FR
    QC = 2
    SEGS = (0, 448, 1152)
    STAGES = (((1, 0, 0), (0, 0, 0)), ((1, 1, 0), (1, 1, 0)), ((2, 2, 2), (2, 2, 2)), ((4, 4, 4), (4, 4, 4)))
    LAG, GO, FSP, CSP, NG = 4, 3, 3, 2, 21
    segs = tuple(zip(SEGS, SEGS[1:] + (QR,)))
    cexp = (DH ** -0.5) * math.log2(math.e)
    porder = [o * 7 + i for o in _ORDER for i in _ORDER]
    SEM_Q, SEM_A = 0, 2 * NQ
    SEM_COLD = SEM_A + 2 * NA
    NSEM = SEM_COLD + len(STAGES) - 1

    def kernel(ax, ak, av, awq, awo, bx, bk, bv, bwq, bwo, out_hbm,
               x_s, k_s, v_s, wq_s, wo_s, q_s, t_s, d_s, m_s, c_s, p_s, out_s, sems):
        src = ((ax, ak, av, awq, awo), (bx, bk, bv, bwq, bwo))
        st = lambda i: i if isinstance(i, int) else 0

        def xb_dma():
            return pltpu.make_async_copy(bx, x_s.at[1], sems.at[SEM_Q + NQ])

        def wq_dmas(br, j, sem):
            return [pltpu.make_async_copy(src[st(br)][3].at[:, pl.ds((st(j) * NS + sl) * SW * DH, SW * DH)],
                                          wq_s.at[br, j, sl], sems.at[sem]) for sl in range(NS)]

        def wo_dmas(br, sl, sem):
            rows = pl.ds(sl * HQ * DH, HQ * DH)
            if sl // NHQ == 0:
                return [pltpu.make_async_copy(src[st(br)][4].at[rows, :], wo_s.at[br, sl],
                                              sems.at[sem])]
            return [pltpu.make_async_copy(src[st(br)][4].at[rows, pl.ds((NB - 1 - nb) * NW, NW)],
                                          wo_s.at[br, sl, :, pl.ds(nb * NW, NW)], sems.at[sem])
                    for nb in range(NB)]

        def kv_dmas(br, j):
            t = br * NA + j
            hs = pl.ds(st(j) * GA, GA)
            return [pltpu.make_async_copy(src[st(br)][1].at[:, hs], k_s.at[t], sems.at[SEM_A + t]),
                    pltpu.make_async_copy(src[st(br)][2].at[:, hs], v_s.at[t], sems.at[SEM_A + t])]

        def out_dma(br, blk, nblk, nb):
            rows = pl.ds(blk * R, nblk * R)
            return pltpu.make_async_copy(out_s.at[br, nb, rows],
                                         out_hbm.at[rows, pl.ds(br * D + nb * NW, NW)], sems.at[SEM_Q + br])

        cold = []
        prev = ((0,) * len(segs),) * NS
        for si, lev in enumerate(STAGES):
            sem = sems.at[SEM_Q if si == 0 else SEM_COLD + si - 1]
            grp = []
            for sl in range(NS):
                if max(lev[sl]) > max(prev[sl]):
                    ks = pl.ds(max(prev[sl]) * DH, (max(lev[sl]) - max(prev[sl])) * DH)
                    grp.append(pltpu.make_async_copy(awq.at[ks, pl.ds(sl * SW * DH, SW * DH)],
                                                     wq_s.at[0, 0, sl, ks], sem))
            for (r0, r1), k0, k1 in zip(segs, map(max, *prev), map(max, *lev)):
                if k1 > k0:
                    idx = (pl.ds(r0, (M if r1 == QR else r1) - r0), pl.ds(k0 * DH, (k1 - k0) * DH))
                    grp.append(pltpu.make_async_copy(ax.at[idx], x_s.at[(0,) + idx], sem))
            cold.append(grp)
            prev = lev
        for grp in cold:
            for d in grp:
                d.start()
        for br in range(2):
            if br == 1:
                xb_dma().start(priority=1)
            for j in range(NQ):
                if br + j == 0:
                    dmas = wo_dmas(0, 0, SEM_Q + 1)
                else:
                    dmas = wq_dmas(br, j, SEM_Q + br * NQ + j) + wo_dmas(br, j, SEM_Q + br * NQ + j)
                for d in dmas:
                    d.start(priority=1)
            for j in range(NA):
                for d in kv_dmas(br, j):
                    d.start(priority=1)

        mask = (lax.broadcasted_iota(jnp.int32, (R, DH), 0) // S
                == lax.broadcasted_iota(jnp.int32, (R, DH), 1) // S)

        def q_proj(br, j, r0, r1, h0, nh):
            w = wq_s[br, j, h0 // SW, :, (h0 % SW) * DH:(h0 % SW + nh) * DH]
            q = jnp.dot(x_s[br, r0:r1, :], w, preferred_element_type=F32)
            for h in range(nh):
                q_s[j, h0 + h, r0:r1, :] = q[:, h * DH:(h + 1) * DH].astype(BF)
            return q

        def t_tile(br, u, r0, gates, always, dacc):
            sl, half = u
            lo = pl.multiple_of(half * DH + r0, TT)
            w = {}
            for kb in range(NB):
                rows = pl.ds(kb * KB + lo, TT)
                for nb in range(NB):
                    w[(kb, nb)] = wo_s[br, sl, rows, nb * NW:(nb + 1) * NW].astype(F32)
            diag = (lax.broadcasted_iota(jnp.int32, (TT, DH), 1)
                    == lax.broadcasted_iota(jnp.int32, (TT, DH), 0) + r0)
            for kb in range(NB):
                a = [jnp.abs(w[(kb, nb)]) for nb in range(NB)]
                d = jnp.sum((a[0] + a[1]) + (a[2] + a[3]), axis=-1, keepdims=True)
                d = jnp.clip(d, 2.0 ** -100, 2.0 ** 100)
                dinv = pl.reciprocal(d, approx=True)
                dinv = dinv * (2.0 - d * dinv)
                for nb in range(NB):
                    w[(kb, nb)] = w[(kb, nb)] * dinv
                part = jnp.where(diag, d, 0.0)
                dacc[kb] = part if r0 == 0 else dacc[kb] + part
                if r0 + TT == DH:
                    drow = jnp.sum(jnp.where(always, dacc[kb], gates[-1]), axis=0, keepdims=True)
                    d_s[sl, kb, half] = jnp.broadcast_to(drow, (8, DH))
            for o in range(7):
                ob = {ii: _signed_sum(lambda oi: w[(oi[0] * 2 + ii[0], oi[1] * 2 + ii[1])], _SB[o])
                      for ii in ((0, 0), (0, 1), (1, 0), (1, 1))}
                for i in range(7):
                    p = o * 7 + i
                    tv = jnp.where(always, _signed_sum(ob.get, _SB_IN[i]), gates[p * len(gates) // NP])
                    t_s[sl, p, pl.ds(lo, TT), :] = tv.astype(BF)

        prev = ((0,) * len(segs),) * NS
        for si, lev in enumerate(STAGES):
            for d in cold[si]:
                d.wait()
            for sl in range(NS):
                for (r0, r1), k0, k1 in zip(segs, prev[sl], lev[sl]):
                    if k1 == k0:
                        continue
                    q = jnp.dot(x_s[0, r0:r1, k0 * DH:k1 * DH], wq_s[0, 0, sl, k0 * DH:k1 * DH, :],
                                preferred_element_type=F32)
                    for h in range(SW):
                        qh = q[:, h * DH:(h + 1) * DH]
                        if k0 > 0:
                            qh = qh + c_s[sl, h, r0:r1, :]
                        if k1 * DH < D:
                            c_s[sl, h, r0:r1, :] = qh
                        else:
                            q_s[0, sl * SW + h, r0:r1, :] = qh.astype(BF)
            prev = lev
        for d in wo_dmas(0, 0, SEM_Q + 1):
            d.wait()

        def q_body(j, br):
            sem = SEM_Q + br * NQ + j
            for d in wq_dmas(br, j, sem):
                d.wait()
            pltpu.make_async_copy(wo_s.at[br, j], wo_s.at[br, j], sems.at[sem]).wait()
            rc = QR // QC
            tiles = [(k, r0) for k in range(TPI) for r0 in range(0, DH, TT)]
            per = len(tiles) // (NS * QC)
            slots = [(nt, r_) for nt in range(SW) for r_ in range(0, rc - TT + 1, TT)]
            always = j >= 0
            us = [jnp.where(br == 0, jnp.minimum((j - 1) * TPI + k, NTU - 1), 2 * j + min(k, 1))
                  for k in range(TPI)]
            us = [(u >> 1, u & 1) for u in us]
            dacc = {}
            for qi in range(NS * QC):
                h0, ri = (qi // QC) * SW, qi % QC
                q = q_proj(br, j, ri * rc, (ri + 1) * rc, h0, SW)
                for ti, (k, r0) in enumerate(tiles[qi * per:(qi + 1) * per]):
                    gates = []
                    for gi in range(NG):
                        nt, r_ = slots[(ti * NG + gi) * len(slots) // (per * NG)]
                        gates.append(q[r_:r_ + TT, nt * DH:(nt + 1) * DH])
                    t_tile(br, us[k], r0, gates, always, dacc)
            return br

        def ao_body(j, br):
            t = br * NA + j
            for d in kv_dmas(br, j):
                d.wait()
            always, step0 = j >= 0, j == 0
            final = [t == b_ * NA + NA - 1 for b_ in range(2)]
            sub = [j * NHQ + i for i in range(NHQ)]
            zpad = jnp.zeros((DH - R, DH), BF)
            chunks = [(ci, hq) for ci in range(NC) for hq in range(NHQ)]
            units = [(ci * NB + p, hq * HQ + h)
                     for (ci, hq) in chunks for p in range(NB) for h in range(HQ)]
            upc = NB * HQ
            soft, outs, hist, lastm = {}, {}, [], {}
            pending, cqueue, cdone, ctick = [], [], set(), [0]

            def qk(u):
                p, h = units[u]
                kk = jnp.concatenate([k_s[t, 2 * p:2 * p + 2, h].reshape(R, DH), zpad], axis=0)
                s = lax.dot_general(q_s[sub[h // GQ], h % GQ, p * R:(p + 1) * R, :], kk, _NT,
                                    preferred_element_type=F32)
                s = jnp.where(mask, s, -jnp.inf)
                e = jnp.exp2((s - jnp.max(s, axis=-1, keepdims=True)) * cexp)
                soft[u] = (e, pl.reciprocal(jnp.sum(e, axis=-1, keepdims=True), approx=True))

            def pv(u):
                p, h = units[u]
                vv = jnp.concatenate([v_s[t, 2 * p:2 * p + 2, h].reshape(R, DH), zpad], axis=0)
                e, rinv = soft.pop(u)
                if len(hist) >= GO:
                    e = jnp.where(always, e, hist[-GO])
                o = jnp.dot(e.astype(BF), vv, preferred_element_type=F32) * rinv
                o = o * d_s[sub[h // HQ], h % HQ // HPB, h % HPB, 0:1, :]
                hist.append(o)
                outs[(p, h)] = o

            def recombine(ci, rb, nb, terms, first, last, gate):
                rows = pl.ds((ci * NB + rb) * R, R)
                if first:
                    cv = jnp.where(step0, 0.0, c_s[0, NB - 1 - nb, rows, :])
                else:
                    cv = p_s[nb, pl.ds(rb * R, R), :]
                if gate is not None:
                    cv = jnp.where(always, cv, gate)
                for p, sgn in terms:
                    mv = lastm[p] if p in lastm else m_s[p, pl.ds((ci % 2) * R, R), :]
                    cv = cv + mv if sgn > 0 else cv - mv
                if not last:
                    p_s[nb, pl.ds(rb * R, R), :] = cv
                    return
                c_s[j, nb, rows, :] = cv
                out_s[br, NB - 1 - nb, rows, :] = cv.astype(BF)
                cdone.add((ci, rb, nb))
                g = 1 if ci == NC - 1 else NB
                r0 = rb // g * g
                if all((ci, r_, nb) in cdone for r_ in range(r0, r0 + g)):
                    for b_ in range(2):
                        @pl.when(final[b_])
                        def _():
                            out_dma(b_, ci * NB + r0, g, NB - 1 - nb).start()

            def product(u, p):
                ci, hq = chunks[u]
                last_chunk = u == len(chunks) - 1
                blk = lambda idx: jnp.concatenate(
                    [outs[(ci * NB + idx[0], hq * HQ + idx[1] * HPB + h)] for h in range(HPB)], axis=1)
                a = _signed_sum(blk, _lhs_terms(p)).astype(BF)
                mv = jnp.dot(a, t_s[sub[hq], p], preferred_element_type=F32)
                ctick[0] += 1
                if cqueue and (ctick[0] >= CSP or last_chunk):
                    ctick[0] = 0
                    recombine(*cqueue.pop(0), mv)
                assert all(task[0] >= ci - 1 for task in cqueue)
                rs = pl.ds((ci % 2) * R, R)
                if hq > 0:
                    mv = mv + m_s[p, rs, :]
                if last_chunk and p in porder[-2:]:
                    assert all(task[0] == ci for task in cqueue)
                    lastm[p] = mv
                else:
                    m_s[p, rs, :] = mv
                if hq < NHQ - 1:
                    return
                o_, i_ = divmod(p, 7)
                for oblk, oterms in _SC.items():
                    oseq = sorted(oterms, key=lambda x: _ORDER.index(x[0]))
                    for pos, (ko, so) in enumerate(oseq):
                        if ko != o_:
                            continue
                        for iblk, iterms in _SC_IN.items():
                            iseq = sorted(iterms, key=lambda x: _ORDER.index(x[0]))
                            if iseq[-1][0] == i_:
                                cqueue.append((ci, oblk[0] * 2 + iblk[0], oblk[1] * 2 + iblk[1],
                                               [(o_ * 7 + ki, so * si) for ki, si in iseq],
                                               pos == 0, pos == len(oseq) - 1))

            fill = list(range(GA))
            tick = [0]

            def filler():
                if fill and tick[0] % FSP == 0:
                    h = fill.pop(0)
                    q_proj(br, sub[h // GQ], QR, M, h % GQ, 1)
                tick[0] += 1

            for u in range(LAG):
                filler()
                qk(u)
            credit = 0.0
            for u in range(len(units)):
                filler()
                pv(u)
                if u + LAG < len(units):
                    assert not fill or (units[u + LAG][0] + 1) * R <= QR
                    qk(u + LAG)
                if (u + 1) % upc == 0:
                    pending += [(u // upc, p) for p in porder]
                credit += NP / upc
                n = int(credit + 1e-9)
                credit -= n
                for _ in range(min(n, len(pending))):
                    product(*pending.pop(0))
            while pending:
                product(*pending.pop(0))
            while cqueue:
                recombine(*cqueue.pop(0), None)
            return br

        def branch(br, carry):
            @pl.when(br == 1)
            def _():
                xb_dma().wait()
            lax.fori_loop(1 - br, NQ, q_body, br)
            lax.fori_loop(0, NA, ao_body, br)
            return carry

        lax.fori_loop(0, 2, branch, 0)
        for b_ in range(2):
            for nb in range(NB):
                for ci in range(NC - 1):
                    out_dma(b_, ci * NB, NB, nb).wait()
                for rb in range(NB):
                    out_dma(b_, (NC - 1) * NB + rb, 1, nb).wait()

    anyspec = pl.BlockSpec(memory_space=pl.ANY)
    out = pl.pallas_call(
        kernel,
        in_specs=[anyspec] * 10,
        out_specs=anyspec,
        out_shape=jax.ShapeDtypeStruct((M, 2 * D), BF),
        scratch_shapes=[
            pltpu.VMEM((2, M, D), BF),
            pltpu.VMEM((2 * NA, B, GA, S, DH), BF),
            pltpu.VMEM((2 * NA, B, GA, S, DH), BF),
            pltpu.VMEM((2, NQ, NS, D, SW * DH), BF),
            pltpu.VMEM((2, NSL, HQ * DH, D), BF),
            pltpu.VMEM((NQ, GQ, M, DH), BF),
            pltpu.VMEM((NSL, NP, KB, NW), BF),
            pltpu.VMEM((NSL, NB, HPB, 8, DH), F32),
            pltpu.VMEM((NP, 2 * R, NW), F32),
            pltpu.VMEM((NA, NB, M, NW), F32),
            pltpu.VMEM((NB, NB * R, NW), F32),
            pltpu.VMEM((2, NB, M, NW), BF),
            pltpu.SemaphoreType.DMA((NSEM,)),
        ],
        compiler_params=pltpu.CompilerParams(vmem_limit_bytes=120 * 1024 * 1024),
    )(A_x.reshape(M, D), A_k_cache, A_v_cache, A_wq, A_wo,
      B_x.reshape(M, D), B_k_cache, B_v_cache, B_wq, B_wo)
    return out.reshape(B, S, 2 * D)
```

```python
import math

import jax
import jax.numpy as jnp
from jax import lax
import jax.experimental.pallas as pl
import jax.experimental.pallas.tpu as pltpu

F32 = jnp.float32
BF = jnp.bfloat16
_NT = (((1,), (1,)), ((), ()))

_SA = [[((0, 0), 1), ((1, 1), -1)], [((1, 0), 1), ((1, 1), -1)], [((0, 0), 1)], [((1, 1), 1)],
       [((0, 0), 1), ((0, 1), -1)], [((1, 0), 1), ((0, 0), -1)], [((1, 1), 1), ((0, 1), -1)]]
_SB = [[((0, 0), 1), ((1, 1), 1)], [((0, 0), 1)], [((0, 1), 1), ((1, 1), 1)], [((1, 0), 1), ((0, 0), 1)],
       [((1, 1), 1)], [((0, 0), 1), ((0, 1), -1)], [((1, 1), 1), ((1, 0), -1)]]
_SC = {(0, 0): [(0, 1), (3, 1), (4, -1), (6, 1)], (0, 1): [(2, 1), (4, -1)],
       (1, 0): [(1, 1), (3, 1)], (1, 1): [(0, -1), (1, 1), (2, 1), (5, -1)]}
_SA_IN = [[((0, 0), 1), ((1, 1), 1)], [((1, 0), 1), ((1, 1), 1)], [((0, 0), 1)], [((1, 1), 1)],
          [((0, 0), 1), ((0, 1), 1)], [((1, 0), 1), ((0, 0), -1)], [((0, 1), 1), ((1, 1), -1)]]
_SB_IN = [[((0, 0), 1), ((1, 1), -1)], [((0, 0), 1)], [((0, 1), 1), ((1, 1), -1)], [((1, 0), 1), ((0, 0), -1)],
          [((1, 1), 1)], [((0, 0), 1), ((0, 1), -1)], [((1, 0), 1), ((1, 1), -1)]]
_SC_IN = {(0, 0): [(0, 1), (3, 1), (4, 1), (6, 1)], (0, 1): [(2, 1), (4, 1)],
          (1, 0): [(1, 1), (3, 1)], (1, 1): [(0, -1), (1, 1), (2, 1), (5, -1)]}
_ORDER = [2, 4, 0, 3, 6, 1, 5]


def _lhs_terms(p):
    t = [((o[0] * 2 + i[0], o[1] * 2 + i[1]), so * si)
         for (o, so) in _SA[p // 7] for (i, si) in _SA_IN[p % 7]]
    return [t[0], t[3], t[1], t[2]] if len(t) == 4 else t


def _signed_sum(get, terms):
    assert terms[0][1] > 0
    acc = get(terms[0][0])
    for idx, sgn in terms[1:]:
        acc = acc + get(idx) if sgn > 0 else acc - get(idx)
    return acc


@jax.jit
def pallas_concat_heads__gqa_block_cached__gqa_block_cached__near_ridge_kernel(
    A_x: jax.Array,
    A_k_cache: jax.Array,
    A_v_cache: jax.Array,
    A_wq: jax.Array,
    A_wo: jax.Array,
    B_x: jax.Array,
    B_k_cache: jax.Array,
    B_v_cache: jax.Array,
    B_wq: jax.Array,
    B_wo: jax.Array,
):
    B, S, D = A_x.shape
    _, H, SK, DH = A_k_cache.shape
    assert (B, S, D, H, SK, DH) == (32, 48, 512, 32, 48, 128) and A_wq.shape == (D, H * DH)
    M = B * S
    R = 2 * S
    GQ, SW = 8, 4
    GA, HQ = 16, 8
    NQ, NS, NA, NHQ, NSL = H // GQ, GQ // SW, H // GA, GA // HQ, H // HQ
    assert GQ == HQ and NA == 2 and NS == NA
    NB, NP = 4, 49
    NC = M // (NB * R)
    KB, NW, HPB = HQ * DH // NB, D // NB, HQ // NB
    TT = 16
    NTU, TPI = 2 * NSL, 3
    FR = 160
    QR = M - FR
    QC = 2
    SEGS = (0, 448, 1152)
    STAGES = (((1, 0, 0), (0, 0, 0)), ((1, 1, 0), (1, 1, 0)), ((2, 2, 2), (2, 2, 2)), ((4, 4, 4), (4, 4, 4)))
    LAG, GO, FSP, CSP, NG = 4, 3, 3, 2, 21
    segs = tuple(zip(SEGS, SEGS[1:] + (QR,)))
    cexp = (DH ** -0.5) * math.log2(math.e)
    porder = [o * 7 + i for o in _ORDER for i in _ORDER]
    SEM_Q, SEM_A = 0, 2 * NQ
    SEM_XB = SEM_A + 2 * NA
    SEM_COLD = SEM_XB + 1
    NSEM = SEM_COLD + len(STAGES)

    def kernel(ax, ak, av, awq, awo, bx, bk, bv, bwq, bwo, out_hbm,
               x_s, k_s, v_s, wq_s, wo_s, q_s, t_s, d_s, m_s, c_s, p_s, out_s, sems):
        src = ((ax, ak, av, awq, awo), (bx, bk, bv, bwq, bwo))
        st = lambda i: i if isinstance(i, int) else 0

        def xb_dma():
            return pltpu.make_async_copy(bx, x_s.at[1], sems.at[SEM_XB])

        def wq_dmas(br, j, sem):
            return [pltpu.make_async_copy(src[st(br)][3].at[:, pl.ds((st(j) * NS + sl) * SW * DH, SW * DH)],
                                          wq_s.at[br, j, sl], sems.at[sem]) for sl in range(NS)]

        def wo_dmas(br, sl, sem):
            rows = pl.ds(sl * HQ * DH, HQ * DH)
            if sl // NHQ == 0:
                return [pltpu.make_async_copy(src[st(br)][4].at[rows, :], wo_s.at[br, sl],
                                              sems.at[sem])]
            return [pltpu.make_async_copy(src[st(br)][4].at[rows, pl.ds((NB - 1 - nb) * NW, NW)],
                                          wo_s.at[br, sl, :, pl.ds(nb * NW, NW)], sems.at[sem])
                    for nb in range(NB)]

        def kv_dmas(br, j):
            t = br * NA + j
            hs = pl.ds(st(j) * GA, GA)
            return [pltpu.make_async_copy(src[st(br)][1].at[:, hs], k_s.at[t], sems.at[SEM_A + t]),
                    pltpu.make_async_copy(src[st(br)][2].at[:, hs], v_s.at[t], sems.at[SEM_A + t])]

        def out_dma(br, blk, nblk, nb):
            rows = pl.ds(blk * R, nblk * R)
            return pltpu.make_async_copy(out_s.at[br, nb, rows],
                                         out_hbm.at[rows, pl.ds(br * D + nb * NW, NW)],
                                         sems.at[SEM_COLD + br])

        cold = []
        prev = ((0,) * len(segs),) * NS
        for si, lev in enumerate(STAGES):
            sem = sems.at[SEM_COLD + si]
            grp = []
            for sl in range(NS):
                if max(lev[sl]) > max(prev[sl]):
                    ks = pl.ds(max(prev[sl]) * DH, (max(lev[sl]) - max(prev[sl])) * DH)
                    grp.append(pltpu.make_async_copy(awq.at[ks, pl.ds(sl * SW * DH, SW * DH)],
                                                     wq_s.at[0, 0, sl, ks], sem))
            for (r0, r1), k0, k1 in zip(segs, map(max, *prev), map(max, *lev)):
                if k1 > k0:
                    idx = (pl.ds(r0, (M if r1 == QR else r1) - r0), pl.ds(k0 * DH, (k1 - k0) * DH))
                    grp.append(pltpu.make_async_copy(ax.at[idx], x_s.at[(0,) + idx], sem))
            cold.append(grp)
            prev = lev
        for grp in cold:
            for d in grp:
                d.start()
        for br in range(2):
            if br == 1:
                xb_dma().start(priority=1)
            for j in range(NQ):
                sem = SEM_Q + br * NQ + j
                for d in (wq_dmas(br, j, sem) if br + j else []) + wo_dmas(br, j, sem):
                    d.start(priority=1)
            for j in range(NA):
                for d in kv_dmas(br, j):
                    d.start(priority=1)

        mask = (lax.broadcasted_iota(jnp.int32, (R, DH), 0) // S
                == lax.broadcasted_iota(jnp.int32, (R, DH), 1) // S)

        def q_proj(br, j, r0, r1, h0, nh):
            w = wq_s[br, j, h0 // SW, :, (h0 % SW) * DH:(h0 % SW + nh) * DH]
            q = jnp.dot(x_s[br, r0:r1, :], w, preferred_element_type=F32)
            for h in range(nh):
                q_s[j, h0 + h, r0:r1, :] = q[:, h * DH:(h + 1) * DH].astype(BF)
            return q

        def t_tile(br, u, r0, gates, always, dacc):
            sl, half = u
            lo = pl.multiple_of(half * DH + r0, TT)
            w = {}
            for kb in range(NB):
                rows = pl.ds(kb * KB + lo, TT)
                for nb in range(NB):
                    w[(kb, nb)] = wo_s[br, sl, rows, nb * NW:(nb + 1) * NW].astype(F32)
            diag = (lax.broadcasted_iota(jnp.int32, (TT, DH), 1)
                    == lax.broadcasted_iota(jnp.int32, (TT, DH), 0) + r0)
            for kb in range(NB):
                a = [jnp.abs(w[(kb, nb)]) for nb in range(NB)]
                d = jnp.sum((a[0] + a[1]) + (a[2] + a[3]), axis=-1, keepdims=True)
                d = jnp.clip(d, 2.0 ** -100, 2.0 ** 100)
                dinv = pl.reciprocal(d, approx=True)
                dinv = dinv * (2.0 - d * dinv)
                for nb in range(NB):
                    w[(kb, nb)] = w[(kb, nb)] * dinv
                part = jnp.where(diag, d, 0.0)
                dacc[kb] = part if r0 == 0 else dacc[kb] + part
                if r0 + TT == DH:
                    drow = jnp.sum(jnp.where(always, dacc[kb], gates[-1]), axis=0, keepdims=True)
                    d_s[sl, kb, half] = jnp.broadcast_to(drow, (8, DH))
            for o in range(7):
                ob = {ii: _signed_sum(lambda oi: w[(oi[0] * 2 + ii[0], oi[1] * 2 + ii[1])], _SB[o])
                      for ii in ((0, 0), (0, 1), (1, 0), (1, 1))}
                for i in range(7):
                    p = o * 7 + i
                    tv = jnp.where(always, _signed_sum(ob.get, _SB_IN[i]), gates[p * len(gates) // NP])
                    t_s[sl, p, pl.ds(lo, TT), :] = tv.astype(BF)

        prev = ((0,) * len(segs),) * NS
        for si, lev in enumerate(STAGES):
            for d in cold[si]:
                d.wait()
            for sl in range(NS):
                for (r0, r1), k0, k1 in zip(segs, prev[sl], lev[sl]):
                    if k1 == k0:
                        continue
                    q = jnp.dot(x_s[0, r0:r1, k0 * DH:k1 * DH], wq_s[0, 0, sl, k0 * DH:k1 * DH, :],
                                preferred_element_type=F32)
                    for h in range(SW):
                        qh = q[:, h * DH:(h + 1) * DH]
                        if k0 > 0:
                            qh = qh + c_s[sl, h, r0:r1, :]
                        if k1 * DH < D:
                            c_s[sl, h, r0:r1, :] = qh
                        else:
                            q_s[0, sl * SW + h, r0:r1, :] = qh.astype(BF)
            prev = lev
        for d in wo_dmas(0, 0, SEM_Q):
            d.wait()

        def q_body(j, br):
            sem = SEM_Q + br * NQ + j
            for d in wq_dmas(br, j, sem):
                d.wait()
            pltpu.make_async_copy(wo_s.at[br, j], wo_s.at[br, j], sems.at[sem]).wait()
            rc = QR // QC
            tiles = [(k, r0) for k in range(TPI) for r0 in range(0, DH, TT)]
            per = len(tiles) // (NS * QC)
            slots = [(nt, r_) for nt in range(SW) for r_ in range(0, rc - TT + 1, TT)]
            always = j >= 0
            us = [jnp.where(br == 0, jnp.minimum((j - 1) * TPI + k, NTU - 1), 2 * j + min(k, 1))
                  for k in range(TPI)]
            us = [(u >> 1, u & 1) for u in us]
            dacc = {}
            for qi in range(NS * QC):
                h0, ri = (qi // QC) * SW, qi % QC
                q = q_proj(br, j, ri * rc, (ri + 1) * rc, h0, SW)
                for ti, (k, r0) in enumerate(tiles[qi * per:(qi + 1) * per]):
                    gates = []
                    for gi in range(NG):
                        nt, r_ = slots[(ti * NG + gi) * len(slots) // (per * NG)]
                        gates.append(q[r_:r_ + TT, nt * DH:(nt + 1) * DH])
                    t_tile(br, us[k], r0, gates, always, dacc)
            return br

        def ao_body(j, br):
            t = br * NA + j
            for d in kv_dmas(br, j):
                d.wait()
            always, step0 = j >= 0, j == 0
            final = [t == b_ * NA + NA - 1 for b_ in range(2)]
            sub = [j * NHQ + i for i in range(NHQ)]
            zpad = jnp.zeros((DH - R, DH), BF)
            chunks = [(ci, hq) for ci in range(NC) for hq in range(NHQ)]
            units = [(ci * NB + p, hq * HQ + h)
                     for (ci, hq) in chunks for p in range(NB) for h in range(HQ)]
            upc = NB * HQ
            soft, outs, hist, lastm = {}, {}, [], {}
            pending, cqueue, cdone, ctick = [], [], set(), [0]

            def qk(u):
                p, h = units[u]
                kk = jnp.concatenate([k_s[t, 2 * p:2 * p + 2, h].reshape(R, DH), zpad], axis=0)
                s = lax.dot_general(q_s[sub[h // GQ], h % GQ, p * R:(p + 1) * R, :], kk, _NT,
                                    preferred_element_type=F32)
                s = jnp.where(mask, s, -jnp.inf)
                e = jnp.exp2((s - jnp.max(s, axis=-1, keepdims=True)) * cexp)
                soft[u] = (e, pl.reciprocal(jnp.sum(e, axis=-1, keepdims=True), approx=True))

            def pv(u):
                p, h = units[u]
                vv = jnp.concatenate([v_s[t, 2 * p:2 * p + 2, h].reshape(R, DH), zpad], axis=0)
                e, rinv = soft.pop(u)
                if len(hist) >= GO:
                    e = jnp.where(always, e, hist[-GO])
                o = jnp.dot(e.astype(BF), vv, preferred_element_type=F32) * rinv
                o = o * d_s[sub[h // HQ], h % HQ // HPB, h % HPB, 0:1, :]
                hist.append(o)
                outs[(p, h)] = o

            def recombine(ci, rb, nb, terms, first, last, gate):
                rows = pl.ds((ci * NB + rb) * R, R)
                if first:
                    cv = jnp.where(step0, 0.0, c_s[0, NB - 1 - nb, rows, :])
                else:
                    cv = p_s[nb, pl.ds(rb * R, R), :]
                if gate is not None:
                    cv = jnp.where(always, cv, gate)
                for p, sgn in terms:
                    mv = lastm[p] if p in lastm else m_s[p, pl.ds((ci % 2) * R, R), :]
                    cv = cv + mv if sgn > 0 else cv - mv
                if not last:
                    p_s[nb, pl.ds(rb * R, R), :] = cv
                    return
                c_s[j, nb, rows, :] = cv
                out_s[br, NB - 1 - nb, rows, :] = cv.astype(BF)
                cdone.add((ci, rb, nb))
                g = 1 if ci == NC - 1 else NB
                r0 = rb // g * g
                if all((ci, r_, nb) in cdone for r_ in range(r0, r0 + g)):
                    for b_ in range(2):
                        @pl.when(final[b_])
                        def _():
                            out_dma(b_, ci * NB + r0, g, NB - 1 - nb).start()

            def product(u, p):
                ci, hq = chunks[u]
                last_chunk = u == len(chunks) - 1
                blk = lambda idx: jnp.concatenate(
                    [outs[(ci * NB + idx[0], hq * HQ + idx[1] * HPB + h)] for h in range(HPB)], axis=1)
                a = _signed_sum(blk, _lhs_terms(p)).astype(BF)
                mv = jnp.dot(a, t_s[sub[hq], p], preferred_element_type=F32)
                ctick[0] += 1
                if cqueue and (ctick[0] >= CSP or last_chunk):
                    ctick[0] = 0
                    recombine(*cqueue.pop(0), mv)
                assert all(task[0] >= ci - 1 for task in cqueue)
                rs = pl.ds((ci % 2) * R, R)
                if hq > 0:
                    mv = mv + m_s[p, rs, :]
                if last_chunk and p in porder[-2:]:
                    assert all(task[0] == ci for task in cqueue)
                    lastm[p] = mv
                else:
                    m_s[p, rs, :] = mv
                if hq < NHQ - 1:
                    return
                o_, i_ = divmod(p, 7)
                for oblk, oterms in _SC.items():
                    oseq = sorted(oterms, key=lambda x: _ORDER.index(x[0]))
                    for pos, (ko, so) in enumerate(oseq):
                        if ko != o_:
                            continue
                        for iblk, iterms in _SC_IN.items():
                            iseq = sorted(iterms, key=lambda x: _ORDER.index(x[0]))
                            if iseq[-1][0] == i_:
                                cqueue.append((ci, oblk[0] * 2 + iblk[0], oblk[1] * 2 + iblk[1],
                                               [(o_ * 7 + ki, so * si) for ki, si in iseq],
                                               pos == 0, pos == len(oseq) - 1))

            fill = list(range(GA))
            tick = [0]

            def filler():
                if fill and tick[0] % FSP == 0:
                    h = fill.pop(0)
                    q_proj(br, sub[h // GQ], QR, M, h % GQ, 1)
                tick[0] += 1

            for u in range(LAG):
                filler()
                qk(u)
            credit = 0.0
            for u in range(len(units)):
                filler()
                pv(u)
                if u + LAG < len(units):
                    assert not fill or (units[u + LAG][0] + 1) * R <= QR
                    qk(u + LAG)
                if (u + 1) % upc == 0:
                    pending += [(u // upc, p) for p in porder]
                credit += NP / upc
                n = int(credit + 1e-9)
                credit -= n
                for _ in range(min(n, len(pending))):
                    product(*pending.pop(0))
            while pending:
                product(*pending.pop(0))
            while cqueue:
                recombine(*cqueue.pop(0), None)
            return br

        def branch(br, carry):
            @pl.when(br == 1)
            def _():
                xb_dma().wait()
            lax.fori_loop(1 - br, NQ, q_body, br)
            lax.fori_loop(0, NA, ao_body, br)
            return carry

        lax.fori_loop(0, 2, branch, 0)
        for b_ in range(2):
            for nb in range(NB):
                for ci in range(NC - 1):
                    out_dma(b_, ci * NB, NB, nb).wait()
                for rb in range(NB):
                    out_dma(b_, (NC - 1) * NB + rb, 1, nb).wait()

    anyspec = pl.BlockSpec(memory_space=pl.ANY)
    out = pl.pallas_call(
        kernel,
        in_specs=[anyspec] * 10,
        out_specs=anyspec,
        out_shape=jax.ShapeDtypeStruct((M, 2 * D), BF),
        scratch_shapes=[
            pltpu.VMEM((2, M, D), BF),
            pltpu.VMEM((2 * NA, B, GA, S, DH), BF),
            pltpu.VMEM((2 * NA, B, GA, S, DH), BF),
            pltpu.VMEM((2, NQ, NS, D, SW * DH), BF),
            pltpu.VMEM((2, NSL, HQ * DH, D), BF),
            pltpu.VMEM((NQ, GQ, M, DH), BF),
            pltpu.VMEM((NSL, NP, KB, NW), BF),
            pltpu.VMEM((NSL, NB, HPB, 8, DH), F32),
            pltpu.VMEM((NP, 2 * R, NW), F32),
            pltpu.VMEM((NA, NB, M, NW), F32),
            pltpu.VMEM((NB, NB * R, NW), F32),
            pltpu.VMEM((2, NB, M, NW), BF),
            pltpu.SemaphoreType.DMA((NSEM,)),
        ],
        compiler_params=pltpu.CompilerParams(vmem_limit_bytes=120 * 1024 * 1024),
    )(A_x.reshape(M, D), A_k_cache, A_v_cache, A_wq, A_wo,
      B_x.reshape(M, D), B_k_cache, B_v_cache, B_wq, B_wo)
    return out.reshape(B, S, 2 * D)
```
